```python
import jax
import jax.numpy as jnp

def _softmax(x, axis=-1):
    return jax.nn.softmax(x, axis=axis)
def _gelu(x):
    return jax.nn.gelu(x, approximate=True)
def _silu(x):
    return jax.nn.silu(x)
def _sigmoid(x):
    return jax.nn.sigmoid(x)
def _layernorm(x, axis=-1, eps=1e-5):
    m = jnp.mean(x, axis=axis, keepdims=True)
    v = jnp.var(x, axis=axis, keepdims=True)
    return (x - m) / jnp.sqrt(v + eps)
def _scatter_add(tgt, idx, src, axis=0):
    return tgt.at[idx].add(src)
def _segment_sum(src, seg, n):
    return jax.ops.segment_sum(src, seg, n)
class _Rng:
    def __init__(self, key):
        self._k = key
    def _next(self):
        self._k, sub = jax.random.split(self._k)
        return sub
    def normal(self, shape):
        return jax.random.normal(self._next(), shape, dtype=jnp.bfloat16)
    def randint(self, lo, hi, shape):
        return jax.random.randint(self._next(), shape, lo, hi, dtype=jnp.int32)
    def uniform(self, shape, lo=0.0, hi=1.0):
        return jax.random.uniform(self._next(), shape, jnp.bfloat16, lo, hi)
    def permutation(self, n):
        return jax.random.permutation(self._next(), n)


kernel_name = 'standalone__modern_conv_block_convnext__vision'

def setup_inputs():
    _rng = _Rng(jax.random.key(int.from_bytes(__import__("os").urandom(4), "little")))
    _w = (lambda a: (lambda t: t.astype(jnp.bfloat16) if jnp.issubdtype(t.dtype, jnp.floating) else t)(jnp.asarray(a)))
    H = W = 512
    C = 96
    K = 3
    return {
        "x": _w((lambda *s: _rng.normal(s) * 0.05)(1, H, W, C)),
        "dw": _w((lambda *s: _rng.normal(s) * 0.05)(K, K, C)),
        "w1": _w((lambda *s: _rng.normal(s) * 0.05)(C, 4 * C)),
        "b1": _w((lambda *s: _rng.normal(s) * 0.05)(4 * C)),
        "w2": _w((lambda *s: _rng.normal(s) * 0.05)(4 * C, C)),
        "b2": _w((lambda *s: _rng.normal(s) * 0.05)(C)),
        "gamma": _w((lambda *s: _rng.normal(s) * 0.05)(C)),
    }

def reference(x, dw, w1, b1, w2, b2, gamma):
    B, H, W, C = x.shape
    K = dw.shape[0]
    pad = K // 2
    xp = jnp.pad(x, ((0,0),(pad,pad),(pad,pad),(0,0)))
    out = jnp.zeros_like(x)
    for i in range(K):
        for j in range(K):
            out = out + xp[:, i:i+H, j:j+W, :] * dw[i, j][None, None, None, :]
    h = _layernorm(out, axis=-1)
    h = jnp.einsum('bhwc,ce->bhwe', h, w1) + b1
    h = _gelu(h)
    h = jnp.einsum('bhwe,ec->bhwc', h, w2) + b2
    return x + gamma[None, None, None, :] * h
```

```python
import functools
import numpy as np
import jax
import jax.numpy as jnp
import jax.experimental.pallas as pl
import jax.experimental.pallas.tpu as pltpu

F32 = jnp.float32
BF16 = jnp.bfloat16
U32 = jnp.uint32

H = W = 512
C = 96
E = 384
NT = W // 128
NC = C // 8
R = 4
C2 = float(np.sqrt(2.0/np.pi) * 0.044715)
GA = float(C2 ** (1.0/3.0))
GK = float(np.sqrt(2.0/np.pi) / GA)
EPS = 1e-5
NXB = 3
NOB = 3


def _tr(a):
    return a.T


def make_kernel(opts):
    order = opts.get('order', 'A')

    def kernel(x_hbm, dw_ref, w1_ref, b1_ref, w2t_ref, b2_ref, g_ref, o_hbm,
               xbuf, obuf, ring0, ring1, ring2, ring3, cb0, cb1, xn0, xn1, gb0, gb1,
               wdw, w1t, w2s, bias2, isem, osem):
        ring = [ring0, ring1, ring2, ring3]
        cb = [cb0, cb1]
        xn = [xn0, xn1]
        gb = [gb0, gb1]
        NG = H // R

        def in_copy(g, slot):
            return pltpu.make_async_copy(x_hbm.at[pl.ds(g * R, R)], xbuf.at[pl.ds(slot * R, R)], isem.at[slot])

        def out_copy(g, slot):
            return pltpu.make_async_copy(obuf.at[pl.ds(slot * R, R)], o_hbm.at[pl.ds(g * R, R)], osem.at[slot])

        in_copy(0, 1 % NXB).start()
        in_copy(1, 2 % NXB).start()

        dwp = dw_ref[...].astype(F32).reshape(9, C)
        dwp = jnp.concatenate([dwp, jnp.zeros((128 - 9, C), F32)], axis=0)
        dwp = jnp.concatenate([dwp, jnp.zeros((128, 128 - C), F32)], axis=1)
        dwt = dwp.T
        for k in range(9):
            wdw[k] = jnp.broadcast_to(dwt[:C, k:k + 1], (C, 128))
        w1 = w1_ref[...].astype(F32)
        w1c = w1 - jnp.mean(w1, axis=0, keepdims=True)
        b1 = b1_ref[...].astype(F32).reshape(1, E) * GA
        bh = b1.astype(BF16).astype(F32)
        bl = b1 - bh
        ext = jnp.concatenate([bh, bl, jnp.zeros((128 - C - 2, E), F32)], axis=0)
        w1a = jnp.concatenate([w1c, ext], axis=0)
        w1t[...] = pltpu.bitcast(w1a.T.astype(BF16), U32)
        gam = g_ref[...].astype(F32).reshape(1, C)
        gb2 = gam * b2_ref[...].astype(F32).reshape(1, C)
        gg = jnp.concatenate([gam * (0.5 / GA), gb2, jnp.zeros((126, C), F32)], axis=0)
        gg = jnp.concatenate([gg, jnp.zeros((128, 128 - C), F32)], axis=1)
        ggt = gg.T
        gcol = jnp.broadcast_to(ggt[:C, 0:1], (C, E))
        w2s[...] = pltpu.bitcast((w2t_ref[...].astype(F32) * gcol).astype(BF16), U32)
        bias2[...] = jnp.broadcast_to(ggt[:C, 1:2], (C, 128))
        rowi = jax.lax.broadcasted_iota(jnp.int32, (32, W), 0)
        cst = jnp.where(rowi < 2, 1.0, 0.0).astype(BF16)
        xn0[C // 2:64, :] = pltpu.bitcast(cst, U32)
        xn1[C // 2:64, :] = pltpu.bitcast(cst, U32)
        xbuf[R - 1] = jnp.zeros((C, W), BF16)

        lane = jax.lax.broadcasted_iota(jnp.int32, (8, 128), 1)
        m0 = lane == 0
        m127 = lane == 127

        def conv_ln(xrow_idx, rnew, r1, r0, cbuf, xnb):
            S = [None] * NT
            Q = [None] * NT
            for c2 in range(NC // 2):
                for hh in range(2):
                    c0 = c2 * 16 + hh * 8
                    cs = pl.ds(c0, 8)
                    xin = xbuf[xrow_idx, cs, :].astype(F32)
                    rnew[cs, :] = xin
                    w = [wdw[k, cs, :] for k in range(9)]
                    s0, s1, s2 = [], [], []
                    for t in range(NT):
                        ls = pl.ds(t * 128, 128)
                        a = r0[cs, ls]
                        b = r1[cs, ls]
                        c = xin[:, t * 128:(t + 1) * 128]
                        s0.append(pltpu.roll(a * w[0] + b * w[3] + c * w[6], 1, 1))
                        s1.append(a * w[1] + b * w[4] + c * w[7])
                        s2.append(pltpu.roll(a * w[2] + b * w[5] + c * w[8], 127, 1))
                    for t in range(NT):
                        l = jnp.where(m0, s0[t - 1] if t > 0 else 0.0, s0[t])
                        r = jnp.where(m127, s2[t + 1] if t < NT - 1 else 0.0, s2[t])
                        o = s1[t] + l + r
                        cbuf[cs, pl.ds(t * 128, 128)] = o
                        if S[t] is None:
                            S[t] = o
                            Q[t] = o * o
                        else:
                            S[t] = S[t] + o
                            Q[t] = Q[t] + o * o
            for t in range(NT):
                ls = pl.ds(t * 128, 128)
                mean = jnp.sum(S[t], axis=0, keepdims=True) * (1.0 / C)
                var = jnp.sum(Q[t], axis=0, keepdims=True) * (1.0 / C) - mean * mean
                r = jax.lax.rsqrt(jnp.maximum(var, 0.0) + EPS) * GA
                for c2 in range(NC // 2):
                    xnb[pl.ds(c2 * 8, 8), ls] = pltpu.bitcast((cbuf[pl.ds(c2 * 16, 16), ls] * r).astype(BF16), U32)

        def mm1(xnb, gbuf):
            h = jnp.dot(pltpu.bitcast(w1t[...], BF16), pltpu.bitcast(xnb[...], BF16), preferred_element_type=F32)
            z = h * (h * h + GK)
            g = (jnp.tanh(z) + 1.0) * h
            gbuf[...] = pltpu.bitcast(g.astype(BF16), U32)

        def mm2(gbuf, rres, orow_idx):
            y = jnp.dot(pltpu.bitcast(w2s[...], BF16), pltpu.bitcast(gbuf[...], BF16), preferred_element_type=F32)
            for c2 in range(NC):
                cs = pl.ds(c2 * 8, 8)
                b = bias2[cs, :]
                b = jnp.concatenate([b] * NT, axis=1)
                obuf[orow_idx, cs, :] = (y[c2 * 8:c2 * 8 + 8, :] + rres[cs, :] + b).astype(BF16)

        in_copy(0, 1 % NXB).wait()

        def body(gi, carry):
            g = gi - 1
            s_cur = gi % NXB
            s_nxt = (gi + 1) % NXB
            oslot = gi % NOB

            @pl.when(jnp.logical_and(gi >= 1, gi + 1 < NG))
            def _():
                in_copy(gi + 1, (gi + 2) % NXB).start()

            @pl.when(jnp.logical_and(gi >= 1, gi < NG))
            def _():
                in_copy(gi, s_nxt).wait()

            @pl.when(gi == NG)
            def _():
                xbuf[s_nxt * R] = jnp.zeros((C, W), BF16)

            @pl.when(gi >= NOB + 1)
            def _():
                out_copy(gi - 1 - NOB, oslot).wait()

            for k in range(R):
                if k == 0:
                    xidx = s_cur * R + 3
                else:
                    xidx = s_nxt * R + (k - 1)
                for st in order:
                    if st == 'c':
                        conv_ln(xidx, ring[(k + 3) % 4], ring[(k + 2) % 4], ring[(k + 1) % 4], cb[k % 2], xn[k % 2])
                    elif st == '1':
                        mm1(xn[(k + 1) % 2], gb[(k + 1) % 2])
                    elif st == '2':
                        mm2(gb[k % 2], ring[k % 4], oslot * R + k)

            @pl.when(gi > 0)
            def _():
                out_copy(gi - 1, oslot).start()
            return carry

        jax.lax.fori_loop(0, NG + 1, body, 0)
        for gi in range(NG + 1 - NOB, NG + 1):
            out_copy(gi - 1, gi % NOB).wait()

    return kernel


def build(opts, name="cnx"):
    kern = make_kernel(opts)

    def f(x, dw, w1, b1, w2, b2, gamma):
        xt = jnp.transpose(x, (0, 1, 3, 2)).reshape(H, C, W)
        out = pl.pallas_call(
            kern,
            out_shape=jax.ShapeDtypeStruct((H, C, W), BF16),
            in_specs=[pl.BlockSpec(memory_space=pl.ANY)] + [pl.BlockSpec(memory_space=pltpu.VMEM)] * 6,
            out_specs=pl.BlockSpec(memory_space=pl.ANY),
            scratch_shapes=[
                pltpu.VMEM((NXB * R, C, W), BF16), pltpu.VMEM((NOB * R, C, W), BF16)]
                + [pltpu.VMEM((C, W), F32)] * 6
                + [pltpu.VMEM((64, W), U32)] * 2
                + [pltpu.VMEM((E // 2, W), U32)] * 2
                + [pltpu.VMEM((9, C, 128), F32), pltpu.VMEM((E // 2, 128), U32), pltpu.VMEM((C // 2, E), U32),
                   pltpu.VMEM((C, 128), F32),
                   pltpu.SemaphoreType.DMA((NXB,)), pltpu.SemaphoreType.DMA((NOB,))],
            compiler_params=pltpu.CompilerParams(vmem_limit_bytes=64 * 1024 * 1024),
            name=name,
        )(xt, dw, w1, b1, w2.T, b2, gamma)
        return jnp.transpose(out.reshape(1, H, C, W), (0, 1, 3, 2))
    return f


_impl = build({'order':'12c'})


@jax.jit
def pallas_standalone__modern_conv_block_convnext__vision_kernel(x, dw, w1, b1, w2, b2, gamma):
    return _impl(x, dw, w1, b1, w2, b2, gamma)
```

```python
import functools
import numpy as np
import jax
import jax.numpy as jnp
from jax import lax
import jax.experimental.pallas as pl
import jax.experimental.pallas.tpu as pltpu

F32 = jnp.float32
BF16 = jnp.bfloat16
U32 = jnp.uint32

H = W = 512
C = 96
E = 384
NT = W // 128
NC = C // 8
R = 8
HR = 4
RS = 8
C2 = float(np.sqrt(2.0/np.pi) * 0.044715)
GA = float(C2 ** (1.0/3.0))
GK = float(np.sqrt(2.0/np.pi) / GA)
EPS = 1e-5
NXB = 3
NOB = 3
DN = (((1,), (0,)), ((), ()))


def make_kernel(opts):
    gmode = opts.get('gmode', 0)
    cvs = opts.get('cvs', 1)
    cts = opts.get('cts', 0)
    order = opts.get('order', 'c12')
    xmode = opts.get('xmode', 1)
    il = opts.get('il', 0)
    gs_ = 0 if gmode == 0 else 1
    CV = gs_ + cvs
    CT = CV + 1 + cts
    assert CT + 1 <= RS
    OFF = 4
    assert CT <= OFF

    def kernel(x_hbm, dw_ref, w1_ref, b1_ref, w2t_ref, b2_ref, g_ref, o_hbm,
               xbuf, obuf, ring, cb, rb, xnb, gbuf, yb, wdw, cst, w1t, w2s, bias2, isem, osem):
        NG = H // R

        def in_copy(g, slot):
            return pltpu.make_async_copy(x_hbm.at[pl.ds(g * R, R)], xbuf.at[pl.ds(slot * R, R)], isem.at[slot])

        def out_copy(i, slot, half):
            return pltpu.make_async_copy(obuf.at[pl.ds(slot * R + half * HR, HR)],
                                         o_hbm.at[pl.ds(i * R - HR + half * HR, HR)], osem.at[slot * 2 + half])

        in_copy(0, 0).start()
        in_copy(1, 1).start()

        dwp = dw_ref[...].astype(F32).reshape(9, C)
        dwp = jnp.concatenate([dwp, jnp.zeros((128 - 9, C), F32)], axis=0)
        dwp = jnp.concatenate([dwp, jnp.zeros((128, 128 - C), F32)], axis=1)
        dwt = dwp.T
        for k in range(9):
            wdw[k] = jnp.broadcast_to(dwt[:C, k:k + 1], (C, 128))
        w1 = w1_ref[...].astype(F32)
        w1c = w1 - jnp.mean(w1, axis=0, keepdims=True)
        b1 = b1_ref[...].astype(F32).reshape(1, E) * GA
        bh = b1.astype(BF16).astype(F32)
        bl = b1 - bh
        ext = jnp.concatenate([bh, bl, jnp.zeros((128 - C - 2, E), F32)], axis=0)
        w1a = jnp.concatenate([w1c, ext], axis=0)
        w1t[...] = pltpu.bitcast(w1a.T.astype(BF16), U32)
        gam = g_ref[...].astype(F32).reshape(1, C)
        gb2 = gam * b2_ref[...].astype(F32).reshape(1, C)
        gg = jnp.concatenate([gam * (0.5 / GA), gb2, jnp.zeros((126, C), F32)], axis=0)
        gg = jnp.concatenate([gg, jnp.zeros((128, 128 - C), F32)], axis=1)
        ggt = gg.T
        gcol = jnp.broadcast_to(ggt[:C, 0:1], (C, E))
        w2s[...] = pltpu.bitcast((w2t_ref[...].astype(F32) * gcol).astype(BF16), U32)
        bias2[...] = jnp.broadcast_to(ggt[:C, 1:2], (C, 128))
        rowi = jax.lax.broadcasted_iota(jnp.int32, (32, 128), 0)
        cst[...] = jnp.where(rowi < 2, 1.0, 0.0)
        ring[RS - 1] = jnp.zeros((C, W), F32)
        for p_ in range(2):
            xnb[p_, C:128, :] = jnp.concatenate([cst[...]] * NT, axis=1)

        lane = jax.lax.broadcasted_iota(jnp.int32, (8, 128), 1)
        m0 = lane == 0
        m127 = lane == 127

        def cvt(xidx, slot):
            for c in range(NC):
                ring[slot, pl.ds(c * 8, 8), :] = xbuf[xidx, pl.ds(c * 8, 8), :].astype(F32)

        def conv(sl2, sl1, sl0, par):
            for _ in convg(sl2, sl1, sl0, par):
                pass

        def convg(sl2, sl1, sl0, par):
            S = [None] * NT
            Q = [None] * NT

            def cst_(k, t, o):
                cb[par, pl.ds(k * 8, 8), pl.ds(t * 128, 128)] = o
                if S[t] is None:
                    S[t] = o
                    Q[t] = o * o
                else:
                    S[t] = S[t] + o
                    Q[t] = Q[t] + o * o
            for k in range(NC):
                cs = pl.ds(k * 8, 8)
                w = [wdw[i, cs, :] for i in range(9)]
                for t in range(NT):
                    ls = pl.ds(t * 128, 128)
                    a = ring[sl0, cs, ls]
                    b = ring[sl1, cs, ls]
                    c = ring[sl2, cs, ls]
                    r0 = pltpu.roll(a * w[0] + b * w[3] + c * w[6], 1, 1)
                    s1 = a * w[1] + b * w[4] + c * w[7]
                    l2 = pltpu.roll(a * w[2] + b * w[5] + c * w[8], 127, 1)
                    if t == 0:
                        p = s1 + jnp.where(m0, 0.0, r0)
                    else:
                        cst_(k, t - 1, pp + jnp.where(m127, l2, pl2))
                        p = s1 + jnp.where(m0, pr0, r0)
                    if t == NT - 1:
                        cst_(k, t, p + jnp.where(m127, 0.0, l2))
                    pp, pr0, pl2 = p, r0, l2
                yield k
            for t in range(NT):
                mean = jnp.sum(S[t], axis=0, keepdims=True) * (1.0 / C)
                var = jnp.sum(Q[t], axis=0, keepdims=True) * (1.0 / C) - mean * mean
                r = jax.lax.rsqrt(jnp.maximum(var, 0.0) + EPS) * GA
                if xmode == 0:
                    ls = pl.ds(t * 128, 128)
                    xnb[par, 0:C, ls] = cb[par, :, ls] * r
                else:
                    rb[par, :, pl.ds(t * 128, 128)] = jnp.broadcast_to(r, (8, 128))

        def xnval(par):
            if xmode == 0:
                return xnb[par]
            r = rb[par]
            c32 = cst[...]
            return jnp.concatenate(
                [cb[par, pl.ds(c * 8, 8), :] * r for c in range(NC)] + [jnp.concatenate([c32] * NT, axis=1)], axis=0)

        def mm1p(xn, m0_, mlen):
            return lax.dot_general(pltpu.bitcast(w1t[pl.ds(m0_ // 2, mlen // 2), :], BF16), xn, DN,
                                   preferred_element_type=F32)

        def mm1(par):
            return mm1p(xnval(par), 0, E)

        def mm1_old(par):
            r = rb[par]
            c32 = cst[...]
            xn = jnp.concatenate(
                [cb[par, pl.ds(c * 8, 8), :] * r for c in range(NC)] + [jnp.concatenate([c32] * NT, axis=1)], axis=0)
            return lax.dot_general(pltpu.bitcast(w1t[...], BF16), xn, DN, preferred_element_type=F32)

        def gelu(hj):
            z = hj * (hj * hj + GK)
            return (jnp.tanh(z) + 1.0) * hj

        def mm2(kt, g, rslot, par, oidx):
            y = lax.dot_general(pltpu.bitcast(w2s[:, kt * 128:(kt + 1) * 128], BF16), g, DN, preferred_element_type=F32)
            for c in range(NC):
                cs = pl.ds(c * 8, 8)
                yc = y[c * 8:c * 8 + 8, :]
                if kt == 0:
                    b = jnp.concatenate([bias2[cs, :]] * NT, axis=1)
                    yb[par, cs, :] = yc + ring[rslot, cs, :] + b
                elif kt == 1:
                    yb[par, cs, :] = yc + yb[par, cs, :]
                else:
                    obuf[oidx, cs, :] = (yc + yb[par, cs, :]).astype(BF16)

        def body(gi, carry):
            s_cur = gi % NXB
            oslot = gi % NOB

            @pl.when(jnp.logical_and(gi >= 1, gi + 1 < NG))
            def _():
                in_copy(gi + 1, (gi + 1) % NXB).start()

            @pl.when(gi < NG)
            def _():
                in_copy(gi, s_cur).wait()

            @pl.when(gi == NG)
            def _():
                xbuf[s_cur * R] = jnp.zeros((C, W), BF16)

            @pl.when(gi >= NOB + 1)
            def _():
                out_copy(gi - NOB, oslot, 0).wait()

            @pl.when(gi >= NOB)
            def _():
                out_copy(gi - NOB, oslot, 1).wait()

            for k in range(R):
                s = k - OFF
                if il:
                    kk = k + CT - OFF
                    xidx = s_cur * R + kk
                    cg = convg((s + CV + 1) % RS, (s + CV) % RS, (s + CV - 1) % RS, (s + CV) % 2)
                    if il & 4:
                        cvt(xidx, (s + CT) % RS)
                    xn = xnval((s + 1) % 2)
                    for kt in range(3):
                        if il & 8:
                            xn = xnval((s + 1) % 2)
                        h = mm1p(xn, kt * 128, 128)
                        gbuf[(s + 1) % 2, pl.ds(kt * 128, 128), :] = gelu(h)
                        if kt == 0 and not (il & 4):
                            cvt(xidx, (s + CT) % RS)
                        if (il & 3) == 1:
                            for _ in range(4):
                                next(cg, None)
                        mm2(kt, gbuf[s % 2, pl.ds(kt * 128, 128), :], s % RS, s % 2, oslot * R + k)
                        if (il & 3) == 2:
                            for _ in range(4):
                                next(cg, None)
                    for _ in cg:
                        pass
                    continue
                for st in order:
                    if st == 'c':
                        kk = k + CT - OFF
                        if kk >= 0:
                            cvt(s_cur * R + kk, (s + CT) % RS)
                        else:
                            cvt(((gi + NXB - 1) % NXB) * R + kk + R, (s + CT) % RS)
                        conv((s + CV + 1) % RS, (s + CV) % RS, (s + CV - 1) % RS, (s + CV) % 2)
                    elif st == '1':
                        h = mm1((s + gs_) % 2)
                        if gmode == 0:
                            for kt in range(3):
                                mm2(kt, gelu(h[kt * 128:(kt + 1) * 128, :]), s % RS, s % 2, oslot * R + k)
                        elif gmode == 1:
                            gbuf[(s + 1) % 2] = gelu(h)
                        else:
                            gbuf[(s + 1) % 2] = pltpu.bitcast(gelu(h).astype(BF16), U32)
                    elif st == '2' and gmode != 0:
                        for kt in range(3):
                            if gmode == 1:
                                g = gbuf[s % 2, pl.ds(kt * 128, 128), :]
                            else:
                                g = pltpu.bitcast(gbuf[s % 2, pl.ds(kt * 64, 64), :], BF16)
                            mm2(kt, g, s % RS, s % 2, oslot * R + k)

            @pl.when(gi > 0)
            def _():
                out_copy(gi, oslot, 0).start()

            @pl.when(gi < NG)
            def _():
                out_copy(gi, oslot, 1).start()
            return carry

        jax.lax.fori_loop(0, NG + 1, body, 0)
        for gi in range(NG + 1 - NOB, NG + 1):
            out_copy(gi, gi % NOB, 0).wait()
            if gi < NG:
                out_copy(gi, gi % NOB, 1).wait()

    return kernel


def build(opts, name="cnx"):
    kern = make_kernel(opts)

    def f(x, dw, w1, b1, w2, b2, gamma):
        xt = jnp.transpose(x, (0, 1, 3, 2)).reshape(H, C, W)
        out = pl.pallas_call(
            kern,
            out_shape=jax.ShapeDtypeStruct((H, C, W), BF16),
            in_specs=[pl.BlockSpec(memory_space=pl.ANY)] + [pl.BlockSpec(memory_space=pltpu.VMEM)] * 6,
            out_specs=pl.BlockSpec(memory_space=pl.ANY),
            scratch_shapes=[
                pltpu.VMEM((NXB * R, C, W), BF16), pltpu.VMEM((NOB * R, C, W), BF16),
                pltpu.VMEM((RS, C, W), F32), pltpu.VMEM((2, C, W), F32), pltpu.VMEM((2, 8, W), F32), pltpu.VMEM((2, 128, W), F32),
                pltpu.VMEM((2, E // 2, W), U32) if opts.get('gmode') == 2 else pltpu.VMEM((2, E, W), F32),
                pltpu.VMEM((2, C, W), F32),
                pltpu.VMEM((9, C, 128), F32), pltpu.VMEM((32, 128), F32),
                pltpu.VMEM((E // 2, 128), U32), pltpu.VMEM((C // 2, E), U32),
                pltpu.VMEM((C, 128), F32),
                pltpu.SemaphoreType.DMA((NXB,)), pltpu.SemaphoreType.DMA((2 * NOB,))],
            compiler_params=pltpu.CompilerParams(vmem_limit_bytes=64 * 1024 * 1024, flags=opts.get('flags')),
            name=name,
        )(xt, dw, w1, b1, w2.T, b2, gamma)
        return jnp.transpose(out.reshape(1, H, C, W), (0, 1, 3, 2))
    return f


_impl = build({'gmode':1,'cvs':1,'cts':1})


@jax.jit
def pallas_standalone__modern_conv_block_convnext__vision_kernel(x, dw, w1, b1, w2, b2, gamma):
    return _impl(x, dw, w1, b1, w2, b2, gamma)
```

```python
import functools
import numpy as np
import jax
import jax.numpy as jnp
from jax import lax
import jax.experimental.pallas as pl
import jax.experimental.pallas.tpu as pltpu

F32 = jnp.float32
BF16 = jnp.bfloat16
U32 = jnp.uint32

H = W = 512
C = 96
E = 384
NT = W // 128
NC = C // 8
C2 = float(np.sqrt(2.0/np.pi) * 0.044715)
GA = float(C2 ** (1.0/3.0))
GK = float(np.sqrt(2.0/np.pi) / GA)
EPS = 1e-5
DN = (((1,), (0,)), ((), ()))


def make_kernel(opts):
    R = opts.get('R', 8)
    cvs = opts.get('cvs', 2)
    cts = opts.get('cts', 1)
    order = opts.get('order', 'tc12')
    xmode = opts.get('xmode', 1)
    gp = opts.get('gp', 0)
    bfly = opts.get('bfly', 1)
    ymode = opts.get('ymode', 2)
    xp = opts.get('xp', 0)
    CV = 1 + cvs
    CT = CV + 1 + cts
    NXB = 3
    NOB = 3
    RS = R
    assert CT + 1 <= RS
    NG = H // R

    def kernel(x_hbm, dw_ref, w1_ref, b1_ref, w2t_ref, b2_ref, g_ref, o_hbm,
               xbuf, obuf, ring, cb, rb, xnb, gbuf, gpk, yb, wdw, cst, w1t, w2s, bias2, isem, osem):

        def in_copy(g, slot):
            return pltpu.make_async_copy(x_hbm.at[pl.ds(g * R, R)], xbuf.at[pl.ds(slot * R, R)], isem.at[slot])

        def out_copy(g, slot):
            return pltpu.make_async_copy(obuf.at[pl.ds(slot * R, R)], o_hbm.at[pl.ds(g * R, R)], osem.at[slot])

        in_copy(0, 0).start()
        in_copy(1, 1).start()

        dwp = dw_ref[...].astype(F32).reshape(9, C)
        dwp = jnp.concatenate([dwp, jnp.zeros((128 - 9, C), F32)], axis=0)
        dwp = jnp.concatenate([dwp, jnp.zeros((128, 128 - C), F32)], axis=1)
        dwt = dwp.T
        for k in range(9):
            wdw[k] = jnp.broadcast_to(dwt[:C, k:k + 1], (C, 128))
        w1 = w1_ref[...].astype(F32)
        w1c = w1 - jnp.mean(w1, axis=0, keepdims=True)
        b1 = b1_ref[...].astype(F32).reshape(1, E) * GA
        bh = b1.astype(BF16).astype(F32)
        bl = b1 - bh
        ext = jnp.concatenate([bh, bl, jnp.zeros((128 - C - 2, E), F32)], axis=0)
        w1a = jnp.concatenate([w1c, ext], axis=0)
        w1t[...] = pltpu.bitcast(w1a.T.astype(BF16), U32)
        gam = g_ref[...].astype(F32).reshape(1, C)
        gb2 = gam * b2_ref[...].astype(F32).reshape(1, C)
        gg = jnp.concatenate([gam * (0.5 / GA), gb2, jnp.zeros((126, C), F32)], axis=0)
        gg = jnp.concatenate([gg, jnp.zeros((128, 128 - C), F32)], axis=1)
        ggt = gg.T
        gcol = jnp.broadcast_to(ggt[:C, 0:1], (C, E))
        w2s[...] = pltpu.bitcast((w2t_ref[...].astype(F32) * gcol).astype(BF16), U32)
        bias2[...] = jnp.broadcast_to(ggt[:C, 1:2], (C, 128))
        rowi = jax.lax.broadcasted_iota(jnp.int32, (32, 128), 0)
        cst[...] = jnp.where(rowi < 2, 1.0, 0.0)
        if xmode == 0:
            for p_ in range(R):
                xnb[p_, C:128, :] = jnp.concatenate([cst[...]] * NT, axis=1)

        sub = jax.lax.broadcasted_iota(jnp.int32, (8, 128), 0)
        lane = jax.lax.broadcasted_iota(jnp.int32, (8, 128), 1)
        m0 = lane == 0
        m127 = lane == 127

        def cvt(xidx, slot, valid):
            for c in range(NC):
                v = xbuf[xidx, pl.ds(c * 8, 8), :].astype(F32)
                if valid is not None:
                    v = jnp.where(valid, v, 0.0)
                ring[slot, pl.ds(c * 8, 8), :] = v

        def conv(sl2, sl1, sl0, par):
            for _ in convg(sl2, sl1, sl0, par):
                pass

        def convg(sl2, sl1, sl0, par):
            S = [None] * NT
            Q = [None] * NT

            def cst_(k, t, o):
                cb[par, pl.ds(k * 8, 8), pl.ds(t * 128, 128)] = o
                if S[t] is None:
                    S[t] = o
                    Q[t] = o * o
                else:
                    S[t] = S[t] + o
                    Q[t] = Q[t] + o * o
            for k in range(NC):
                cs = pl.ds(k * 8, 8)
                w = [wdw[i, cs, :] for i in range(9)]
                for t in range(NT):
                    ls = pl.ds(t * 128, 128)
                    a = ring[sl0, cs, ls]
                    b = ring[sl1, cs, ls]
                    c = ring[sl2, cs, ls]
                    r0 = pltpu.roll(a * w[0] + b * w[3] + c * w[6], 1, 1)
                    s1 = a * w[1] + b * w[4] + c * w[7]
                    l2 = pltpu.roll(a * w[2] + b * w[5] + c * w[8], 127, 1)
                    if t == 0:
                        p = s1 + jnp.where(m0, 0.0, r0)
                    else:
                        cst_(k, t - 1, pp + jnp.where(m127, l2, pl2))
                        p = s1 + jnp.where(m0, pr0, r0)
                    if t == NT - 1:
                        cst_(k, t, p + jnp.where(m127, 0.0, l2))
                    pp, pr0, pl2 = p, r0, l2
                yield k
            if bfly:
                def merge(a, b, d):
                    msk = (sub % (2 * d)) < d
                    return jnp.where(msk, a, b) + pltpu.roll(jnp.where(msk, b, a), 8 - d, 0)
                v = merge(merge(merge(S[0], S[1], 1), merge(S[2], S[3], 1), 2),
                          merge(merge(Q[0], Q[1], 1), merge(Q[2], Q[3], 1), 2), 4) * (1.0 / C)
                var = pltpu.roll(v, 4, 0) - v * v
                r = jax.lax.rsqrt(jnp.maximum(var, 0.0) + EPS) * GA
                rb[par, :, 0:128] = r
                return
            for t in range(NT):
                mean = jnp.sum(S[t], axis=0, keepdims=True) * (1.0 / C)
                var = jnp.sum(Q[t], axis=0, keepdims=True) * (1.0 / C) - mean * mean
                r = jax.lax.rsqrt(jnp.maximum(var, 0.0) + EPS) * GA
                if xmode == 0:
                    ls = pl.ds(t * 128, 128)
                    xnb[par, 0:C, ls] = cb[par, :, ls] * r
                else:
                    rb[par, :, pl.ds(t * 128, 128)] = jnp.broadcast_to(r, (8, 128))

        def xnval(par):
            if xmode == 0:
                return xnb[par]
            if bfly:
                r = jnp.concatenate([jnp.broadcast_to(rb[par, pl.ds(t, 1), 0:128], (8, 128)) for t in range(NT)], axis=1)
            else:
                r = rb[par]
            c32 = cst[...]
            v = jnp.concatenate(
                [cb[par, pl.ds(c * 8, 8), :] * r for c in range(NC)] + [jnp.concatenate([c32] * NT, axis=1)], axis=0)
            return v.astype(BF16) if xp else v

        def gelu(hj):
            z = hj * (hj * hj + GK)
            return (jnp.tanh(z) + 1.0) * hj

        def mm1(par, gsl):
            h = lax.dot_general(pltpu.bitcast(w1t[...], BF16), xnval(par), DN, preferred_element_type=F32)
            if gp == 2:
                g = gelu(h)
                gpk[pl.ds(gsl * (E // 2), E // 2), :] = pltpu.bitcast(g[:, 0:256].astype(BF16), U32)
                gbuf[pl.ds(gsl * E, E), :] = g[:, 256:512]
            elif gp == 3:
                g = gelu(h)
                gpk[pl.ds(gsl * (E // 2), E // 2), :] = pltpu.bitcast(g[:, 0:384].astype(BF16), U32)
                gbuf[pl.ds(gsl * E, E), 0:128] = g[:, 384:512]
            elif gp:
                gbuf[pl.ds(gsl * (E // 2), E // 2), :] = pltpu.bitcast(gelu(h).astype(BF16), U32)
            else:
                gbuf[gsl] = gelu(h)

        def mm2n(gsl, rslot, oidx):
            for _ in mm2g(gsl, rslot, oidx):
                pass

        def mm2g(gsl, rslot, oidx):
            if ymode == 1:
                for kt in range(3):
                    if gp == 1:
                        g = pltpu.bitcast(gbuf[pl.ds(gsl * (E // 2) + kt * 64, 64), :], BF16)
                    else:
                        g = gbuf[gsl, pl.ds(kt * 128, 128), :]
                    y = lax.dot_general(pltpu.bitcast(w2s[:, kt * 128:(kt + 1) * 128], BF16), g, DN,
                                        preferred_element_type=F32)
                    for c in range(NC):
                        cs = pl.ds(c * 8, 8)
                        yc = y[c * 8:c * 8 + 8, :]
                        if kt == 0:
                            b = jnp.concatenate([bias2[cs, :]] * NT, axis=1)
                            yb[gsl, cs, :] = yc + (ring[rslot, cs, :] + b)
                        elif kt == 1:
                            yb[gsl, cs, :] = yc + yb[gsl, cs, :]
                        else:
                            obuf[oidx, cs, :] = (yc + yb[gsl, cs, :]).astype(BF16)
                return
            yield from mm2g2(gsl, rslot, oidx)

        def mm2g2(gsl, rslot, oidx):
            def d(k0, kl, n0):
                if gp == 2:
                    if n0 == 0:
                        g = pltpu.bitcast(gpk[pl.ds(gsl * (E // 2) + k0 // 2, kl // 2), :], BF16)
                    else:
                        g = gbuf[pl.ds(gsl * E + k0, kl), :]
                elif gp:
                    g = pltpu.bitcast(gbuf[pl.ds(gsl * (E // 2) + k0 // 2, kl // 2), pl.ds(n0, 256)], BF16)
                else:
                    g = gbuf[gsl, pl.ds(k0, kl), pl.ds(n0, 256)]
                return lax.dot_general(pltpu.bitcast(w2s[:, k0:k0 + kl], BF16), g, DN, preferred_element_type=F32)

            def fin(n0, ya, k1, kl1):
                ts = []
                for c in range(NC):
                    cs = pl.ds(c * 8, 8)
                    b = jnp.concatenate([bias2[cs, :]] * 2, axis=1)
                    ts.append(ya[c * 8:c * 8 + 8, :] + (ring[rslot, cs, pl.ds(n0, 256)] + b))
                yield
                yb_ = d(k1, kl1, n0)
                for c in range(NC):
                    obuf[oidx, pl.ds(c * 8, 8), pl.ds(n0, 256)] = (ts[c] + yb_[c * 8:c * 8 + 8, :]).astype(BF16)
            a = d(0, 256, 0)
            yield from fin(0, a, 256, 128)
            c_ = d(0, 128, 256)
            yield
            yield from fin(256, c_, 128, 256)

        ring[RS - 1] = jnp.zeros((C, W), F32)
        in_copy(0, 0).wait()

        def pro_cvt(r, c):
            cvt(r, r, None)
            return c
        lax.fori_loop(0, CT, pro_cvt, 0)

        def pro_conv(r, c):
            conv(r + 1, r, (r + RS - 1) % RS, r)
            return c
        lax.fori_loop(0, CV, pro_conv, 0)
        mm1(0, 0)

        def body(gi, carry):
            s0 = gi * R
            sl0 = gi % NXB
            sl1 = (gi + 1) % NXB
            oslot = gi % NOB
            in_copy(jnp.minimum(gi + 2, NG - 1), (gi + 2) % NXB).start()

            @pl.when(gi >= NOB)
            def _():
                out_copy(0, oslot).wait()
            in_copy(0, sl1).wait()

            for k in range(R):
                cg = convg((k + CV + 1) % RS, (k + CV) % RS, (k + CV - 1) % RS, (k + CV) % R)
                yg = mm2g(k % 2, k, oslot * R + k)
                for st in order:
                    if st == 't':
                        kk = k + CT
                        xidx = sl0 * R + kk if kk < R else sl1 * R + kk - R
                        valid = (s0 + kk < H) if kk == R else None
                        cvt(xidx, kk % R, valid)
                    elif st == 'c':
                        for _ in cg:
                            pass
                    elif st in 'hq':
                        for _ in range(6 if st == 'h' else 3):
                            next(cg, None)
                    elif st == '1':
                        mm1((k + 1) % R, (k + 1) % 2)
                    elif st == 'y':
                        next(yg, None)
                    elif st == '2':
                        for _ in yg:
                            pass
                for _ in cg:
                    pass
                for _ in yg:
                    pass
            out_copy(gi, oslot).start()
            return carry

        NGR = opts.get('ng', NG)
        lax.fori_loop(0, NGR, body, 0)
        in_copy(0, (NGR + 1) % NXB).wait()
        for gi in range(NGR - NOB, NGR):
            out_copy(gi, gi % NOB).wait()

    return kernel


def build(opts, name="cnx"):
    kern = make_kernel(opts)
    R = opts.get('R', 8)

    def f(x, dw, w1, b1, w2, b2, gamma):
        xt = jnp.transpose(x, (0, 1, 3, 2)).reshape(H, C, W)
        out = pl.pallas_call(
            kern,
            out_shape=jax.ShapeDtypeStruct((H, C, W), BF16),
            in_specs=[pl.BlockSpec(memory_space=pl.ANY)] + [pl.BlockSpec(memory_space=pltpu.VMEM)] * 6,
            out_specs=pl.BlockSpec(memory_space=pl.ANY),
            scratch_shapes=[
                pltpu.VMEM((3 * R, C, W), BF16), pltpu.VMEM((3 * R, C, W), BF16),
                pltpu.VMEM((R, C, W), F32), pltpu.VMEM((R, C, W), F32), pltpu.VMEM((R, 8, W), F32),
                pltpu.VMEM((R, 128, W) if opts.get('xmode', 1) == 0 else (R, 8, 128), F32),
                pltpu.VMEM((E, W), U32) if opts.get('gp') == 1 else pltpu.VMEM((2 * E, 256), F32) if opts.get('gp') == 2 else pltpu.VMEM((2, E, W), F32),
                pltpu.VMEM((E, 256), U32),
                pltpu.VMEM((2, C, W), F32),
                pltpu.VMEM((9, C, 128), F32), pltpu.VMEM((32, 128), F32),
                pltpu.VMEM((E // 2, 128), U32), pltpu.VMEM((C // 2, E), U32),
                pltpu.VMEM((C, 128), F32),
                pltpu.SemaphoreType.DMA((3,)), pltpu.SemaphoreType.DMA((3,))],
            compiler_params=pltpu.CompilerParams(vmem_limit_bytes=64 * 1024 * 1024, flags=opts.get('flags'),
                                                 disable_bounds_checks=opts.get('dbc', False)),
            name=name,
        )(xt, dw, w1, b1, w2.T, b2, gamma)
        return jnp.transpose(out.reshape(1, H, C, W), (0, 1, 3, 2))
    return f


_impl = build({'dbc':True,'gp':1,'R':16})


@jax.jit
def pallas_standalone__modern_conv_block_convnext__vision_kernel(x, dw, w1, b1, w2, b2, gamma):
    return _impl(x, dw, w1, b1, w2, b2, gamma)
```

```python
import numpy as np
import jax
import jax.numpy as jnp
from jax import lax
import jax.experimental.pallas as pl
import jax.experimental.pallas.tpu as pltpu

F32 = jnp.float32
BF16 = jnp.bfloat16
U32 = jnp.uint32

H = W = 512
C = 96
E = 384
NT = W // 128
NC = C // 8
C2 = float(np.sqrt(2.0 / np.pi) * 0.044715)
GA = float(C2 ** (1.0 / 3.0))
GK = float(np.sqrt(2.0 / np.pi) / GA)
EPS = 1e-5
DN = (((1,), (0,)), ((), ()))
NXB = 2
NOB = 2


def make_kernel(o):
    R = o.get('R', 16)
    CV = 1 + o.get('cvs', 2)
    CT = CV + 1 + o.get('cts', 1)
    OQ = o.get('oq', 4)
    NQ = R // OQ
    NG = H // R
    gp = o.get('gp', 1)
    cs_ = o.get('cs', 0)
    po = o.get('po', 0)
    ko = o.get('ko', 0)
    yo = o.get('yo', 0)
    ge = o.get('ge', 0)
    fo = o.get('fo', 0)
    qo = o.get('qo', 0)
    cw = o.get('cw', 8)
    to = o.get('to', 0)
    gm = o.get('gm', 1)
    pm = o.get('pm', -1)
    fn = o.get('fn', -1)

    def kernel(x_hbm, dw_ref, w1_ref, b1_ref, w2t_ref, b2_ref, g_ref, o_hbm,
               xbuf, obuf, ring, cb, rb, gbuf, gf32, ga0, ga1, g00, g01, g02, g10, g11, g12, zs, wdw, cst, w1t, w2s, bias2, isem, osem):

        class _Multi:
            def __init__(self, cps):
                self.cps = cps

            def start(self):
                for c in self.cps:
                    c.start()

            def wait(self):
                for c in self.cps:
                    c.wait()

        def in_copy(g, slot):
            a0 = jnp.minimum(g * R + CT, H - R + CT)
            b0 = jnp.minimum((g + 1) * R, H - CT)
            return _Multi([
                pltpu.make_async_copy(x_hbm.at[pl.ds(a0, R - CT)], xbuf.at[pl.ds(slot * R, R - CT)], isem.at[2 * slot]),
                pltpu.make_async_copy(x_hbm.at[pl.ds(b0, CT)], xbuf.at[pl.ds(slot * R + R - CT, CT)], isem.at[2 * slot + 1]),
            ])

        def out_copy(g, slot, q):
            return pltpu.make_async_copy(obuf.at[pl.ds(slot * R + q * OQ, OQ)], o_hbm.at[pl.ds(g * R + q * OQ, OQ)],
                                         osem.at[slot * NQ + q])

        first = pltpu.make_async_copy(x_hbm.at[pl.ds(0, CT)], xbuf.at[pl.ds(NXB * R, CT)], isem.at[2 * NXB])
        first.start()
        PK = o.get('peel', 0)
        if PK:
            p0 = pltpu.make_async_copy(x_hbm.at[pl.ds(CT, PK)], xbuf.at[pl.ds(0, PK)], isem.at[0])
            p1 = pltpu.make_async_copy(x_hbm.at[pl.ds(CT + PK, R - PK)], xbuf.at[pl.ds(PK, R - PK)], isem.at[1])
            p0.start()
            p1.start()
        else:
            in_copy(0, 0).start()

        dwp = dw_ref[...].astype(F32).reshape(9, C)
        dwp = jnp.concatenate([dwp, jnp.zeros((128 - 9, C), F32)], axis=0)
        dwp = jnp.concatenate([dwp, jnp.zeros((128, 128 - C), F32)], axis=1)
        dwt = dwp.T
        for k in range(9):
            wdw[k] = jnp.broadcast_to(dwt[:C, k:k + 1], (C, 128))
        w1 = w1_ref[...].astype(F32)
        w1c = w1 - jnp.mean(w1, axis=0, keepdims=True)
        b1 = b1_ref[...].astype(F32).reshape(1, E) * GA
        bh = b1.astype(BF16).astype(F32)
        bl = b1 - bh
        ext = jnp.concatenate([bh, bl, jnp.zeros((128 - C - 2, E), F32)], axis=0)
        w1a = jnp.concatenate([w1c, ext], axis=0)
        w1t[...] = pltpu.bitcast(w1a.T.astype(BF16), U32)
        gam = g_ref[...].astype(F32).reshape(1, C)
        gb2 = gam * b2_ref[...].astype(F32).reshape(1, C)
        gg = jnp.concatenate([gam * (0.5 / GA), gb2, jnp.zeros((126, C), F32)], axis=0)
        gg = jnp.concatenate([gg, jnp.zeros((128, 128 - C), F32)], axis=1)
        ggt = gg.T
        gcol = jnp.broadcast_to(ggt[:C, 0:1], (C, E))
        w2s[...] = pltpu.bitcast((w2t_ref[...].astype(F32) * gcol).astype(BF16), U32)
        bias2[...] = jnp.broadcast_to(ggt[:C, 1:2], (C, 128))
        rowi = jax.lax.broadcasted_iota(jnp.int32, (32, 128), 0)
        cst[...] = jnp.where(rowi < 2, 1.0, 0.0)

        sub = jax.lax.broadcasted_iota(jnp.int32, (8, 128), 0)
        lane = jax.lax.broadcasted_iota(jnp.int32, (8, 128), 1)
        m0 = lane == 0
        m127 = lane == 127
        zs[0] = 0
        zs[1] = 0
        gt = [[g00, g01, g02], [g10, g11, g12]]
        V = {'a': [ga0, ga1], 'b': [ga0, ga1], 'ta': gt, 'tb': gt}

        def cvt(xidx, slot, valid):
            for c in range(C // cw):
                v = xbuf[xidx, pl.ds(c * cw, cw), :].astype(F32)
                if valid is not None:
                    v = jnp.where(valid, v, 0.0)
                ring[slot, pl.ds(c * cw, cw), :] = v

        def tri(a, wa, b, wb, c, wc):
            if cs_ == 0:
                return (a * wa + b * wb) + c * wc
            if cs_ == 1:
                return (c * wc + b * wb) + a * wa
            return a * wa + (b * wb + c * wc)

        def conv(sl2, sl1, sl0, par, fpar=None):
            for _ in convg(sl2, sl1, sl0, par, fpar):
                pass

        def convg(sl2, sl1, sl0, par, fpar=None, m=-1, fa=None, fb=None):
            S = [[None] * NT for _ in range(2)]
            Q = [[None] * NT for _ in range(2)]

            def cst_(k, t, v):
                cb[par, pl.ds(k * 8, 8), pl.ds(t * 128, 128)] = v
                h = (k % 2) if qo == 1 else (k // (NC // 2) if qo == 2 else 0)
                if S[h][t] is None:
                    S[h][t] = v
                    Q[h][t] = v * v
                else:
                    S[h][t] = S[h][t] + v
                    Q[h][t] = Q[h][t] + v * v
            ks = list(range(NC))
            if ko == 1:
                ks = ks[::-1]
            elif ko == 2:
                ks = ks[0::2] + ks[1::2]
            for ki, k in enumerate(ks):
                if ki == m:
                    if fa is not None:
                        for t in range(NT):
                            fa()[pl.ds(64, 8), pl.ds(t * 128, 128)] = pltpu.bitcast(Q[0][t], U32)
                    yield
                cs = pl.ds(k * 8, 8)
                w = [wdw[i, cs, :] for i in range(9)]
                def taps(t):
                    ls = pl.ds(t * 128, 128)
                    a = ring[sl0, cs, ls]
                    b = ring[sl1, cs, ls]
                    c = ring[sl2, cs, ls]
                    wa = o.get('wa', 0)
                    if wa == 0:
                        return (pltpu.roll(tri(a, w[0], b, w[3], c, w[6]), 1, 1), tri(a, w[1], b, w[4], c, w[7]),
                                pltpu.roll(tri(a, w[2], b, w[5], c, w[8]), 127, 1))
                    x0 = pltpu.roll(tri(a, w[0], b, w[3], c, w[6]), 1, 1)
                    x2 = pltpu.roll(tri(a, w[2], b, w[5], c, w[8]), 127, 1)
                    return x0, tri(a, w[1], b, w[4], c, w[7]), x2
                if o.get('cf', 0) == 1:
                    for t in range(NT):
                        r0, s1, l2 = taps(t)
                        if t == 0:
                            p = s1 + jnp.where(m0, 0.0, r0)
                        else:
                            cst_(k, t - 1, pp + jnp.where(m127, l2, pl2))
                            p = s1 + jnp.where(m0, pr0, r0)
                        if t == NT - 1:
                            cst_(k, t, p + jnp.where(m127, 0.0, l2))
                        pp, pr0, pl2 = p, r0, l2
                    continue
                tp = [taps(t) for t in range(NT)]
                r0 = [x[0] for x in tp]
                s1 = [x[1] for x in tp]
                l2 = [x[2] for x in tp]
                ts_ = range(NT) if to == 0 else range(NT - 1, -1, -1)
                for t in ts_:
                    lft = jnp.where(m0, r0[t - 1] if t > 0 else 0.0, r0[t])
                    rgt = jnp.where(m127, l2[t + 1] if t < NT - 1 else 0.0, l2[t])
                    if po == 0:
                        v = (s1[t] + lft) + rgt
                    elif po == 1:
                        v = (lft + rgt) + s1[t]
                    else:
                        v = (s1[t] + rgt) + lft
                    cst_(k, t, v)
            if qo:
                S = [a + b for a, b in zip(*S)]
                Q = [a + b for a, b in zip(*Q)]
            else:
                S, Q = S[0], Q[0]

            def merge(a, b, d):
                msk = (sub % (2 * d)) < d
                return jnp.where(msk, a, b) + pltpu.roll(jnp.where(msk, b, a), 8 - d, 0)
            v = merge(merge(merge(S[0], S[1], 1), merge(S[2], S[3], 1), 2),
                      merge(merge(Q[0], Q[1], 1), merge(Q[2], Q[3], 1), 2), 4)
            if o.get('lv', 0) == 1:
                var = pltpu.roll(v, 4, 0) - (v * (1.0 / C)) * v
                r = jax.lax.rsqrt(jnp.maximum(var, 0.0) + EPS * C) * (GA * float(np.sqrt(C)))
                rb[par] = r
                return
            v = v * (1.0 / C)
            var = pltpu.roll(v, 4, 0) - v * v
            r = jax.lax.rsqrt(jnp.maximum(var, 0.0) + EPS) * GA
            rb[par] = r
            if fb is not None:
                fb()[pl.ds(72, 8), 0:128] = pltpu.bitcast(r, U32)
            if fpar is not None:
                V['b'][fpar][pl.ds(E // 2, 8), 0:128] = pltpu.bitcast(r, U32)

        def xnval(par):
            r = jnp.concatenate([jnp.broadcast_to(rb[par, pl.ds(t, 1), :], (8, 128)) for t in range(NT)], axis=1)
            c32 = cst[...]
            v = jnp.concatenate(
                [cb[par, pl.ds(c * 8, 8), :] * r for c in range(NC)] + [jnp.concatenate([c32] * NT, axis=1)], axis=0)
            return v.astype(BF16) if o.get('xp', 0) else v

        def gelu(hj):
            if ge == 0:
                z = hj * (hj * hj + GK)
                return (jnp.tanh(z) + 1.0) * hj
            if ge == 1:
                z = (hj * hj) * hj + GK * hj if False else hj * (hj * hj + GK)
                return jnp.tanh(z) * hj + hj
            z = (hj * hj + GK) * hj
            return hj * (1.0 + jnp.tanh(z))

        def mm1(par, gsl):
            h = lax.dot_general(pltpu.bitcast(w1t[...], BF16), xnval(par), DN, preferred_element_type=F32)
            if pm >= 0:
                g = gelu(h)
                for j in range(3):
                    gj = g[j * 128:(j + 1) * 128, :]
                    if (pm >> j) & 1:
                        gbuf[pl.ds(gsl * (E // 2) + j * 64, 64), :] = pltpu.bitcast(gj.astype(BF16), U32)
                    else:
                        gf32[pl.ds(gsl * E + j * 128, 128), :] = gj
                return
            if gm == 3:
                gf32[pl.ds(gsl * E, E), :] = h
                return
            g = gelu(h)
            if gp == 2:
                gbuf[pl.ds(gsl * (E // 2), E // 2), 0:256] = pltpu.bitcast(g[:, 0:256].astype(BF16), U32)
                gf32[pl.ds(gsl * E, E), 256:512] = g[:, 256:512]
            elif gp == 1 and fn == 4:
                for j in range(3):
                    V['ta'][gsl][j][pl.ds(0, 64), :] = pltpu.bitcast(g[j * 128:(j + 1) * 128, :].astype(BF16), U32)
            elif gp == 1 and fn >= 0:
                V['a'][gsl][pl.ds(0, E // 2), :] = pltpu.bitcast(g.astype(BF16), U32)
            elif gp == 1:
                gbuf[pl.ds(gsl * (E // 2), E // 2), :] = pltpu.bitcast(g.astype(BF16), U32)
            else:
                gf32[pl.ds(gsl * E, E), :] = g

        def mm2(gsl, rslot, oidx):
            def d(k0, kl, n0):
                if pm >= 0:
                    acc = None
                    for j in range(k0 // 128, (k0 + kl) // 128):
                        if (pm >> j) & 1:
                            g = pltpu.bitcast(gbuf[pl.ds(gsl * (E // 2) + j * 64, 64), pl.ds(n0, 256)], BF16)
                        else:
                            g = gf32[pl.ds(gsl * E + j * 128, 128), pl.ds(n0, 256)]
                        y = lax.dot_general(pltpu.bitcast(w2s[:, j * 128:(j + 1) * 128], BF16), g, DN,
                                            preferred_element_type=F32)
                        acc = y if acc is None else acc + y
                    return acc
                if gm == 3:
                    g = gelu(gf32[pl.ds(gsl * E + k0, kl), pl.ds(n0, 256)])
                    if gp:
                        g = g.astype(BF16)
                elif gp == 1 and fn == 4:
                    g = jnp.concatenate([pltpu.bitcast(V['ta'][gsl][j][pl.ds(0, 64), pl.ds(n0, 256)], BF16)
                                         for j in range(k0 // 128, (k0 + kl) // 128)], axis=0)
                elif gp == 1 and fn >= 0:
                    g = pltpu.bitcast(V['a'][gsl][pl.ds(k0 // 2, kl // 2), pl.ds(n0, 256)], BF16)
                elif gp == 1 or (gp == 2 and n0 == 0):
                    g = pltpu.bitcast(gbuf[pl.ds(gsl * (E // 2) + k0 // 2, kl // 2), pl.ds(n0, 256)], BF16)
                else:
                    g = gf32[pl.ds(gsl * E + k0, kl), pl.ds(n0, 256)]
                return lax.dot_general(pltpu.bitcast(w2s[:, k0:k0 + kl], BF16), g, DN, preferred_element_type=F32)

            def fin(n0, ya, later):
                ts = []
                for c in range(NC):
                    cs = pl.ds(c * 8, 8)
                    b = jnp.concatenate([bias2[cs, :]] * 2, axis=1)
                    res = ring[rslot, cs, pl.ds(n0, 256)]
                    yc = ya[c * 8:c * 8 + 8, :]
                    if fo == 0:
                        ts.append(yc + (res + b))
                    elif fo == 1:
                        ts.append((yc + res) + b)
                    elif fo == 2:
                        ts.append((yc, res + b))
                    else:
                        ts.append((yc + b, res))
                yb_ = later()
                for c in range(NC):
                    yc = yb_[c * 8:c * 8 + 8, :]
                    if fo < 2:
                        v = ts[c] + yc
                    else:
                        v = (ts[c][0] + yc) + ts[c][1]
                    obuf[oidx, pl.ds(c * 8, 8), pl.ds(n0, 256)] = v.astype(BF16)
            if yo >= 4:
                if gp == 1:
                    g = pltpu.bitcast(gbuf[pl.ds(gsl * (E // 2), E // 2), :], BF16)
                else:
                    g = gf32[pl.ds(gsl * E, E), :]
                if yo == 4:
                    y = lax.dot_general(pltpu.bitcast(w2s[...], BF16), g, DN, preferred_element_type=F32)
                else:
                    def dd(k0, kl, t):
                        return lax.dot_general(pltpu.bitcast(w2s[:, k0:k0 + kl], BF16),
                                               g[k0:k0 + kl, t * 128:(t + 1) * 128], DN, preferred_element_type=F32)
                    y0 = dd(0, 384, 0)
                    y1a = dd(0, 128, 1)
                    y1b = dd(128, 256, 1)
                    y2a = dd(0, 256, 2)
                    y2b = dd(256, 128, 2)
                    y3 = dd(0, 384, 3)
                    parts = [(y0, None), (y1a, y1b), (y2a, y2b), (y3, None)]
                for t in range(NT):
                    ls = pl.ds(t * 128, 128)
                    for c2 in range(NC // 2):
                        cs = pl.ds(c2 * 16, 16)
                        rs_ = slice(c2 * 16, c2 * 16 + 16)
                        res = ring[rslot, cs, ls]
                        b = bias2[cs, :]
                        if yo == 4:
                            yc = y[rs_, t * 128:(t + 1) * 128]
                            v = (yc + res) + b if fo == 1 else yc + (res + b)
                        else:
                            pa, pb = parts[t]
                            if pb is None:
                                v = pa[rs_, :] + (res + b)
                            else:
                                v = (pa[rs_, :] + (res + b)) + pb[rs_, :]
                        obuf[oidx, cs, ls] = v.astype(BF16)
                return
            if yo == 0:
                fin(0, d(0, 256, 0), lambda: d(256, 128, 0))
                fin(256, d(0, 128, 256), lambda: d(128, 256, 256))
            elif yo == 1:
                fin(0, d(128, 256, 0), lambda: d(0, 128, 0))
                fin(256, d(256, 128, 256), lambda: d(0, 256, 256))
            elif yo == 2:
                fin(0, d(0, 256, 0), lambda: d(256, 128, 0))
                fin(256, d(256, 128, 256), lambda: d(0, 256, 256))
            else:
                fin(0, d(128, 256, 0), lambda: d(0, 128, 0))
                fin(256, d(0, 128, 256), lambda: d(128, 256, 256))

        ring[R - 1] = jnp.zeros((C, W), F32)
        first.wait()

        def pro_cvt(r, c):
            cvt(NXB * R + r, r, None)
            return c
        lax.fori_loop(0, CT, pro_cvt, 0)

        def pro_conv(r, c):
            conv(r + 1, r, (r + R - 1) % R, r)
            return c
        lax.fori_loop(0, CV, pro_conv, 0)
        mm1(0, 0)

        def body(gi, carry, peeled=False):
            s0 = gi * R
            sl0 = gi % NXB
            oslot = gi % NOB
            if fn >= 0:
                z0 = pl.multiple_of(zs[0] * 8, 8)
                z1 = pl.multiple_of(zs[1] * 8, 8)
                V['a'] = [g_.at[pl.ds(z0, E // 2 + 8)] for g_ in (ga0, ga1)]
                V['b'] = [g_.at[pl.ds(z1, E // 2 + 8)] for g_ in (ga0, ga1)]
                V['ta'] = [[g_.at[pl.ds(z0, 80)] for g_ in r_] for r_ in gt]
                V['tb'] = [[g_.at[pl.ds(z1, 80)] for g_ in r_] for r_ in gt]
                if o.get('nh'):
                    V['b'] = [pltpu.annotate(g_, no_hazard=True) for g_ in V['b']]
            xs_ = 0 if o.get('sx') else sl0
            os_ = 0 if o.get('so') else oslot
            in_copy(jnp.minimum(gi + 1, NG - 1), (gi + 1) % NXB).start()

            if peeled:
                p0.wait()
            else:
                @pl.when(gi >= NOB)
                def _():
                    for q in range(NQ):
                        out_copy(0, oslot, q).wait()
                in_copy(0, sl0).wait()

            for k in range(R):
                kk = k + CT
                if peeled and k == PK:
                    p1.wait()
                valid = (s0 + kk < H) if kk == R else None
                if not o.get('nocvt'):
                    cvt(xs_ * R + k, kk % R, valid)
                if fn < 0:
                    conv((k + CV + 1) % R, (k + CV) % R, (k + CV - 1) % R, (k + CV) % R)
                elif fn == 0:
                    conv((k + CV + 1) % R, (k + CV) % R, (k + CV - 1) % R, (k + CV) % R, k % 2)
                elif fn == 2:
                    conv((k + CV + 1) % R, (k + CV) % R, (k + CV - 1) % R, (k + CV) % R, (k + 1) % 2)
                elif fn == 4:
                    m, jA, jB = o.get('m', 4), o.get('jA', 2), o.get('jB', 0)
                    def mk(kk_):
                        fA = (lambda: V['tb'][kk_ % 2][jA]) if (jA >= 0 and kk_ > 0) else None
                        fB = (lambda: V['tb'][(kk_ + 1) % 2][jB]) if jB >= 0 else None
                        return convg((kk_ + CV + 1) % R, (kk_ + CV) % R, (kk_ + CV - 1) % R, (kk_ + CV) % R, None, m, fA, fB)
                    if k == 0:
                        pend = mk(0)
                        next(pend)
                    for _ in pend:
                        pass
                    if k + 1 < R:
                        pend = mk(k + 1)
                        next(pend)
                elif fn == 3:
                    conv((k + CV + 1) % R, (k + CV) % R, (k + CV - 1) % R, (k + CV) % R, (k + 1) % 2 if k > 0 else None)
                mm1((k + 1) % R, (k + 1) % 2)
                if fn == 1 and k > 0:
                    kp = k - 1
                    conv((kp + CV + 1) % R, (kp + CV) % R, (kp + CV - 1) % R, (kp + CV) % R, k % 2)
                mm2(k % 2, k, os_ * R + k)
                if fn == 1 and k == R - 1:
                    conv((k + CV + 1) % R, (k + CV) % R, (k + CV - 1) % R, (k + CV) % R)
                if (k + 1) % OQ == 0:
                    out_copy(gi, oslot, k // OQ).start()
            return carry

        NGR = o.get('ng', NG)
        if PK:
            body(0, 0, True)
        lax.fori_loop(1 if PK else 0, NGR, body, 0)
        in_copy(0, NGR % NXB).wait()
        for gi in range(NGR - NOB, NGR):
            for q in range(NQ):
                out_copy(gi, gi % NOB, q).wait()

    return kernel


def build(o, name="cnx"):
    kern = make_kernel(o)
    R = o.get('R', 16)
    NQ = R // o.get('oq', 4)

    def f(x, dw, w1, b1, w2, b2, gamma):
        xt = jnp.transpose(x, (0, 1, 3, 2)).reshape(H, C, W)
        out = pl.pallas_call(
            kern,
            out_shape=jax.ShapeDtypeStruct((H, C, W), BF16),
            in_specs=[pl.BlockSpec(memory_space=pl.ANY)] + [pl.BlockSpec(memory_space=pltpu.VMEM)] * 6,
            out_specs=pl.BlockSpec(memory_space=pl.ANY),
            scratch_shapes=[
                pltpu.VMEM((NXB * R + 8, C, W), BF16), pltpu.VMEM((NOB * R, C, W), BF16),
                pltpu.VMEM((R, C, W), F32), pltpu.VMEM((R, C, W), F32), pltpu.VMEM((R, 8, 128), F32),
                pltpu.VMEM((E, W), U32), pltpu.VMEM((2 * E, W), F32),
                pltpu.VMEM((E // 2 + 24, W), U32), pltpu.VMEM((E // 2 + 24, W), U32)] + [pltpu.VMEM((64 + 24, W), U32)] * 6 + [pltpu.SMEM((2,), jnp.int32),
                pltpu.VMEM((9, C, 128), F32), pltpu.VMEM((32, 128), F32),
                pltpu.VMEM((E // 2, 128), U32), pltpu.VMEM((C // 2, E), U32),
                pltpu.VMEM((C, 128), F32),
                pltpu.SemaphoreType.DMA((2 * NXB + 1,)), pltpu.SemaphoreType.DMA((NOB * NQ,))],
            compiler_params=pltpu.CompilerParams(vmem_limit_bytes=100 * 1024 * 1024, flags=o.get('flags'),
                                                 disable_bounds_checks=o.get('dbc', True)),
            name=name,
        )(xt, dw, w1, b1, w2.T, b2, gamma)
        return jnp.transpose(out.reshape(1, H, C, W), (0, 1, 3, 2))
    return f


_impl = build({'R':32,'peel':8,'gp': 1, 'cs': 0, 'po': 1, 'ko': 1, 'yo': 1, 'ge': 0, 'fo': 1, 'qo': 0, 'cw': 8, 'to': 0, 'cvs': 2, 'cts': 3, 'cf': 0, 'lv': 0})


@jax.jit
def pallas_standalone__modern_conv_block_convnext__vision_kernel(x, dw, w1, b1, w2, b2, gamma):
    return _impl(x, dw, w1, b1, w2, b2, gamma)
```

```python
import numpy as np
import jax
import jax.numpy as jnp
from jax import lax
import jax.experimental.pallas as pl
import jax.experimental.pallas.tpu as pltpu

F32 = jnp.float32
BF16 = jnp.bfloat16
U32 = jnp.uint32

H = W = 512
C = 96
E = 384
NT = W // 128
NC = C // 8
C2 = float(np.sqrt(2.0 / np.pi) * 0.044715)
GA = float(C2 ** (1.0 / 3.0))
GK = float(np.sqrt(2.0 / np.pi) / GA)
EPS = 1e-5
DN = (((1,), (0,)), ((), ()))
NXB = 2
NOB = 2


def make_kernel(o):
    R = o.get('R', 16)
    CV = 1 + o.get('cvs', 2)
    CT = CV + 1 + o.get('cts', 1)
    OQ = o.get('oq', 4)
    NQ = R // OQ
    NG = H // R
    gp = o.get('gp', 1)
    cs_ = o.get('cs', 0)
    po = o.get('po', 0)
    ko = o.get('ko', 0)
    yo = o.get('yo', 0)
    ge = o.get('ge', 0)
    fo = o.get('fo', 0)
    qo = o.get('qo', 0)
    cw = o.get('cw', 8)
    to = o.get('to', 0)
    gm = o.get('gm', 1)
    pm = o.get('pm', -1)
    fn = o.get('fn', -1)

    def kernel(x_hbm, dw_ref, w1_ref, b1_ref, w2t_ref, b2_ref, g_ref, o_hbm,
               xbuf, obuf, ring, cb, rb, gbuf, gf32, ga0, ga1, g00, g01, g02, g10, g11, g12, zs, wdw, cst, w1t, w2s, bias2, isem, osem):

        class _Multi:
            def __init__(self, cps):
                self.cps = cps

            def start(self):
                for c in self.cps:
                    c.start()

            def wait(self):
                for c in self.cps:
                    c.wait()

        def in_copy(g, slot):
            a0 = jnp.minimum(g * R + CT, H - R + CT)
            b0 = jnp.minimum((g + 1) * R, H - CT)
            return _Multi([
                pltpu.make_async_copy(x_hbm.at[pl.ds(a0, R - CT)], xbuf.at[pl.ds(slot * R, R - CT)], isem.at[2 * slot]),
                pltpu.make_async_copy(x_hbm.at[pl.ds(b0, CT)], xbuf.at[pl.ds(slot * R + R - CT, CT)], isem.at[2 * slot + 1]),
            ])

        def out_copy(g, slot, q):
            return pltpu.make_async_copy(obuf.at[pl.ds(slot * R + q * OQ, OQ)], o_hbm.at[pl.ds(g * R + q * OQ, OQ)],
                                         osem.at[slot * NQ + q])

        first = pltpu.make_async_copy(x_hbm.at[pl.ds(0, CT)], xbuf.at[pl.ds(NXB * R, CT)], isem.at[2 * NXB])
        first.start()
        PK = o.get('peel', 0)
        if PK:
            p0 = pltpu.make_async_copy(x_hbm.at[pl.ds(CT, PK)], xbuf.at[pl.ds(0, PK)], isem.at[0])
            p1 = pltpu.make_async_copy(x_hbm.at[pl.ds(CT + PK, R - PK)], xbuf.at[pl.ds(PK, R - PK)], isem.at[1])
            p0.start()
            p1.start()
        else:
            in_copy(0, 0).start()

        dwp = dw_ref[...].astype(F32).reshape(9, C)
        dwp = jnp.concatenate([dwp, jnp.zeros((128 - 9, C), F32)], axis=0)
        dwp = jnp.concatenate([dwp, jnp.zeros((128, 128 - C), F32)], axis=1)
        dwt = dwp.T
        for k in range(9):
            wdw[k] = jnp.broadcast_to(dwt[:C, k:k + 1], (C, 128))
        w1 = w1_ref[...].astype(F32)
        w1c = w1 - jnp.mean(w1, axis=0, keepdims=True)
        b1 = b1_ref[...].astype(F32).reshape(1, E) * GA
        bh = b1.astype(BF16).astype(F32)
        bl = b1 - bh
        ext = jnp.concatenate([bh, bl, jnp.zeros((128 - C - 2, E), F32)], axis=0)
        w1a = jnp.concatenate([w1c, ext], axis=0)
        w1t[...] = pltpu.bitcast(w1a.T.astype(BF16), U32)
        gam = g_ref[...].astype(F32).reshape(1, C)
        gb2 = gam * b2_ref[...].astype(F32).reshape(1, C)
        gg = jnp.concatenate([gam * (0.5 / GA), gb2, jnp.zeros((126, C), F32)], axis=0)
        gg = jnp.concatenate([gg, jnp.zeros((128, 128 - C), F32)], axis=1)
        ggt = gg.T
        gcol = jnp.broadcast_to(ggt[:C, 0:1], (C, E))
        w2s[...] = pltpu.bitcast((w2t_ref[...].astype(F32) * gcol).astype(BF16), U32)
        bias2[...] = jnp.broadcast_to(ggt[:C, 1:2], (C, 128))
        rowi = jax.lax.broadcasted_iota(jnp.int32, (32, 128), 0)
        cst[...] = jnp.where(rowi < 2, 1.0, 0.0)

        sub = jax.lax.broadcasted_iota(jnp.int32, (8, 128), 0)
        lane = jax.lax.broadcasted_iota(jnp.int32, (8, 128), 1)
        m0 = lane == 0
        m127 = lane == 127
        zs[0] = 0
        zs[1] = 0
        gt = [[g00, g01, g02], [g10, g11, g12]]
        V = {'a': [ga0, ga1], 'b': [ga0, ga1], 'ta': gt, 'tb': gt}

        def cvt(xidx, slot, valid):
            for c in range(C // cw):
                v = xbuf[xidx, pl.ds(c * cw, cw), :].astype(F32)
                if valid is not None:
                    v = jnp.where(valid, v, 0.0)
                ring[slot, pl.ds(c * cw, cw), :] = v

        def tri(a, wa, b, wb, c, wc):
            if cs_ == 0:
                return (a * wa + b * wb) + c * wc
            if cs_ == 1:
                return (c * wc + b * wb) + a * wa
            return a * wa + (b * wb + c * wc)

        def conv(sl2, sl1, sl0, par, fpar=None):
            for _ in convg(sl2, sl1, sl0, par, fpar):
                pass

        def convg(sl2, sl1, sl0, par, fpar=None, m=-1, fa=None, fb=None):
            S = [[None] * NT for _ in range(2)]
            Q = [[None] * NT for _ in range(2)]

            def cst_(k, t, v):
                cb[par, pl.ds(k * 8, 8), pl.ds(t * 128, 128)] = v
                h = (k % 2) if qo == 1 else (k // (NC // 2) if qo == 2 else 0)
                if S[h][t] is None:
                    S[h][t] = v
                    Q[h][t] = v * v
                else:
                    S[h][t] = S[h][t] + v
                    Q[h][t] = Q[h][t] + v * v
            ks = list(range(NC))
            if ko == 1:
                ks = ks[::-1]
            elif ko == 2:
                ks = ks[0::2] + ks[1::2]
            for ki, k in enumerate(ks):
                if ki == m:
                    if fa is not None:
                        for t in range(NT):
                            fa()[pl.ds(64, 8), pl.ds(t * 128, 128)] = pltpu.bitcast(Q[0][t], U32)
                    yield
                cs = pl.ds(k * 8, 8)
                w = [wdw[i, cs, :] for i in range(9)]
                def taps(t):
                    ls = pl.ds(t * 128, 128)
                    a = ring[sl0, cs, ls]
                    b = ring[sl1, cs, ls]
                    c = ring[sl2, cs, ls]
                    wa = o.get('wa', 0)
                    if wa == 0:
                        return (pltpu.roll(tri(a, w[0], b, w[3], c, w[6]), 1, 1), tri(a, w[1], b, w[4], c, w[7]),
                                pltpu.roll(tri(a, w[2], b, w[5], c, w[8]), 127, 1))
                    x0 = pltpu.roll(tri(a, w[0], b, w[3], c, w[6]), 1, 1)
                    x2 = pltpu.roll(tri(a, w[2], b, w[5], c, w[8]), 127, 1)
                    return x0, tri(a, w[1], b, w[4], c, w[7]), x2
                if o.get('cf', 0) == 1:
                    for t in range(NT):
                        r0, s1, l2 = taps(t)
                        if t == 0:
                            p = s1 + jnp.where(m0, 0.0, r0)
                        else:
                            cst_(k, t - 1, pp + jnp.where(m127, l2, pl2))
                            p = s1 + jnp.where(m0, pr0, r0)
                        if t == NT - 1:
                            cst_(k, t, p + jnp.where(m127, 0.0, l2))
                        pp, pr0, pl2 = p, r0, l2
                    continue
                tp = [taps(t) for t in range(NT)]
                r0 = [x[0] for x in tp]
                s1 = [x[1] for x in tp]
                l2 = [x[2] for x in tp]
                ts_ = range(NT) if to == 0 else range(NT - 1, -1, -1)
                for t in ts_:
                    lft = jnp.where(m0, r0[t - 1] if t > 0 else 0.0, r0[t])
                    rgt = jnp.where(m127, l2[t + 1] if t < NT - 1 else 0.0, l2[t])
                    if po == 0:
                        v = (s1[t] + lft) + rgt
                    elif po == 1:
                        v = (lft + rgt) + s1[t]
                    else:
                        v = (s1[t] + rgt) + lft
                    cst_(k, t, v)
            if qo:
                S = [a + b for a, b in zip(*S)]
                Q = [a + b for a, b in zip(*Q)]
            else:
                S, Q = S[0], Q[0]

            def merge(a, b, d):
                msk = (sub % (2 * d)) < d
                return jnp.where(msk, a, b) + pltpu.roll(jnp.where(msk, b, a), 8 - d, 0)
            v = merge(merge(merge(S[0], S[1], 1), merge(S[2], S[3], 1), 2),
                      merge(merge(Q[0], Q[1], 1), merge(Q[2], Q[3], 1), 2), 4)
            if o.get('lv', 0) == 1:
                var = pltpu.roll(v, 4, 0) - (v * (1.0 / C)) * v
                r = jax.lax.rsqrt(jnp.maximum(var, 0.0) + EPS * C) * (GA * float(np.sqrt(C)))
                rb[par] = r
                return
            v = v * (1.0 / C)
            var = pltpu.roll(v, 4, 0) - v * v
            r = jax.lax.rsqrt(jnp.maximum(var, 0.0) + EPS) * GA
            rb[par] = r
            if fb is not None:
                fb()[pl.ds(72, 8), 0:128] = pltpu.bitcast(r, U32)
            if fpar is not None:
                V['b'][fpar][pl.ds(E // 2, 8), 0:128] = pltpu.bitcast(r, U32)

        def xnval(par):
            r = jnp.concatenate([jnp.broadcast_to(rb[par, pl.ds(t, 1), :], (8, 128)) for t in range(NT)], axis=1)
            c32 = cst[...]
            v = jnp.concatenate(
                [cb[par, pl.ds(c * 8, 8), :] * r for c in range(NC)] + [jnp.concatenate([c32] * NT, axis=1)], axis=0)
            return v.astype(BF16) if o.get('xp', 0) else v

        def gelu(hj):
            if ge == 0:
                z = hj * (hj * hj + GK)
                return (jnp.tanh(z) + 1.0) * hj
            if ge == 1:
                z = (hj * hj) * hj + GK * hj if False else hj * (hj * hj + GK)
                return jnp.tanh(z) * hj + hj
            z = (hj * hj + GK) * hj
            return hj * (1.0 + jnp.tanh(z))

        def mm1(par, gsl):
            h = lax.dot_general(pltpu.bitcast(w1t[...], BF16), xnval(par), DN, preferred_element_type=F32)
            if pm >= 0:
                g = gelu(h)
                for j in range(3):
                    gj = g[j * 128:(j + 1) * 128, :]
                    if (pm >> j) & 1:
                        gbuf[pl.ds(gsl * (E // 2) + j * 64, 64), :] = pltpu.bitcast(gj.astype(BF16), U32)
                    else:
                        gf32[pl.ds(gsl * E + j * 128, 128), :] = gj
                return
            if gm == 3:
                gf32[pl.ds(gsl * E, E), :] = h
                return
            g = gelu(h)
            if gp == 2:
                gbuf[pl.ds(gsl * (E // 2), E // 2), 0:256] = pltpu.bitcast(g[:, 0:256].astype(BF16), U32)
                gf32[pl.ds(gsl * E, E), 256:512] = g[:, 256:512]
            elif gp == 1 and fn == 4:
                for j in range(3):
                    V['ta'][gsl][j][pl.ds(0, 64), :] = pltpu.bitcast(g[j * 128:(j + 1) * 128, :].astype(BF16), U32)
            elif gp == 1 and fn >= 0:
                V['a'][gsl][pl.ds(0, E // 2), :] = pltpu.bitcast(g.astype(BF16), U32)
            elif gp == 1:
                gbuf[pl.ds(gsl * (E // 2), E // 2), :] = pltpu.bitcast(g.astype(BF16), U32)
            else:
                gf32[pl.ds(gsl * E, E), :] = g

        def mm2(gsl, rslot, oidx):
            def d(k0, kl, n0):
                if pm >= 0:
                    acc = None
                    for j in range(k0 // 128, (k0 + kl) // 128):
                        if (pm >> j) & 1:
                            g = pltpu.bitcast(gbuf[pl.ds(gsl * (E // 2) + j * 64, 64), pl.ds(n0, 256)], BF16)
                        else:
                            g = gf32[pl.ds(gsl * E + j * 128, 128), pl.ds(n0, 256)]
                        y = lax.dot_general(pltpu.bitcast(w2s[:, j * 128:(j + 1) * 128], BF16), g, DN,
                                            preferred_element_type=F32)
                        acc = y if acc is None else acc + y
                    return acc
                if gm == 3:
                    g = gelu(gf32[pl.ds(gsl * E + k0, kl), pl.ds(n0, 256)])
                    if gp:
                        g = g.astype(BF16)
                elif gp == 1 and fn == 4:
                    g = jnp.concatenate([pltpu.bitcast(V['ta'][gsl][j][pl.ds(0, 64), pl.ds(n0, 256)], BF16)
                                         for j in range(k0 // 128, (k0 + kl) // 128)], axis=0)
                elif gp == 1 and fn >= 0:
                    g = pltpu.bitcast(V['a'][gsl][pl.ds(k0 // 2, kl // 2), pl.ds(n0, 256)], BF16)
                elif gp == 1 or (gp == 2 and n0 == 0):
                    g = pltpu.bitcast(gbuf[pl.ds(gsl * (E // 2) + k0 // 2, kl // 2), pl.ds(n0, 256)], BF16)
                else:
                    g = gf32[pl.ds(gsl * E + k0, kl), pl.ds(n0, 256)]
                return lax.dot_general(pltpu.bitcast(w2s[:, k0:k0 + kl], BF16), g, DN, preferred_element_type=F32)

            def fin(n0, ya, later):
                ts = []
                for c in range(NC):
                    cs = pl.ds(c * 8, 8)
                    b = jnp.concatenate([bias2[cs, :]] * 2, axis=1)
                    res = ring[rslot, cs, pl.ds(n0, 256)]
                    yc = ya[c * 8:c * 8 + 8, :]
                    if fo == 0:
                        ts.append(yc + (res + b))
                    elif fo == 1:
                        ts.append((yc + res) + b)
                    elif fo == 2:
                        ts.append((yc, res + b))
                    else:
                        ts.append((yc + b, res))
                yb_ = later()
                for c in range(NC):
                    yc = yb_[c * 8:c * 8 + 8, :]
                    if fo < 2:
                        v = ts[c] + yc
                    else:
                        v = (ts[c][0] + yc) + ts[c][1]
                    obuf[oidx, pl.ds(c * 8, 8), pl.ds(n0, 256)] = v.astype(BF16)
            if yo >= 4:
                if gp == 1:
                    g = pltpu.bitcast(gbuf[pl.ds(gsl * (E // 2), E // 2), :], BF16)
                else:
                    g = gf32[pl.ds(gsl * E, E), :]
                if yo == 4:
                    y = lax.dot_general(pltpu.bitcast(w2s[...], BF16), g, DN, preferred_element_type=F32)
                else:
                    def dd(k0, kl, t):
                        return lax.dot_general(pltpu.bitcast(w2s[:, k0:k0 + kl], BF16),
                                               g[k0:k0 + kl, t * 128:(t + 1) * 128], DN, preferred_element_type=F32)
                    y0 = dd(0, 384, 0)
                    y1a = dd(0, 128, 1)
                    y1b = dd(128, 256, 1)
                    y2a = dd(0, 256, 2)
                    y2b = dd(256, 128, 2)
                    y3 = dd(0, 384, 3)
                    parts = [(y0, None), (y1a, y1b), (y2a, y2b), (y3, None)]
                for t in range(NT):
                    ls = pl.ds(t * 128, 128)
                    for c2 in range(NC // 2):
                        cs = pl.ds(c2 * 16, 16)
                        rs_ = slice(c2 * 16, c2 * 16 + 16)
                        res = ring[rslot, cs, ls]
                        b = bias2[cs, :]
                        if yo == 4:
                            yc = y[rs_, t * 128:(t + 1) * 128]
                            v = (yc + res) + b if fo == 1 else yc + (res + b)
                        else:
                            pa, pb = parts[t]
                            if pb is None:
                                v = pa[rs_, :] + (res + b)
                            else:
                                v = (pa[rs_, :] + (res + b)) + pb[rs_, :]
                        obuf[oidx, cs, ls] = v.astype(BF16)
                return
            if yo == 0:
                fin(0, d(0, 256, 0), lambda: d(256, 128, 0))
                fin(256, d(0, 128, 256), lambda: d(128, 256, 256))
            elif yo == 1:
                fin(0, d(128, 256, 0), lambda: d(0, 128, 0))
                fin(256, d(256, 128, 256), lambda: d(0, 256, 256))
            elif yo == 2:
                fin(0, d(0, 256, 0), lambda: d(256, 128, 0))
                fin(256, d(256, 128, 256), lambda: d(0, 256, 256))
            else:
                fin(0, d(128, 256, 0), lambda: d(0, 128, 0))
                fin(256, d(0, 128, 256), lambda: d(128, 256, 256))

        ring[R - 1] = jnp.zeros((C, W), F32)
        first.wait()

        if o.get('upro', 0):
            for r in range(CT):
                cvt(NXB * R + r, r, None)
            for r in range(CV):
                conv(r + 1, r, (r + R - 1) % R, r)
            mm1(0, 0)
        else:
            def pro_cvt(r, c):
                cvt(NXB * R + r, r, None)
                return c
            lax.fori_loop(0, CT, pro_cvt, 0)

            def pro_conv(r, c):
                conv(r + 1, r, (r + R - 1) % R, r)
                return c
            lax.fori_loop(0, CV, pro_conv, 0)
            mm1(0, 0)

        def body(gi, carry, peeled=False):
            s0 = gi * R
            sl0 = gi % NXB
            oslot = gi % NOB
            if fn >= 0:
                z0 = pl.multiple_of(zs[0] * 8, 8)
                z1 = pl.multiple_of(zs[1] * 8, 8)
                V['a'] = [g_.at[pl.ds(z0, E // 2 + 8)] for g_ in (ga0, ga1)]
                V['b'] = [g_.at[pl.ds(z1, E // 2 + 8)] for g_ in (ga0, ga1)]
                V['ta'] = [[g_.at[pl.ds(z0, 80)] for g_ in r_] for r_ in gt]
                V['tb'] = [[g_.at[pl.ds(z1, 80)] for g_ in r_] for r_ in gt]
                if o.get('nh'):
                    V['b'] = [pltpu.annotate(g_, no_hazard=True) for g_ in V['b']]
            xs_ = 0 if o.get('sx') else sl0
            os_ = 0 if o.get('so') else oslot
            in_copy(jnp.minimum(gi + 1, NG - 1), (gi + 1) % NXB).start()

            if peeled:
                p0.wait()
            else:
                @pl.when(gi >= NOB)
                def _():
                    for q in range(NQ):
                        out_copy(0, oslot, q).wait()
                in_copy(0, sl0).wait()

            for k in range(R):
                kk = k + CT
                if peeled and k == PK:
                    p1.wait()
                valid = (s0 + kk < H) if kk == R else None
                if not o.get('nocvt'):
                    cvt(xs_ * R + k, kk % R, valid)
                if fn < 0:
                    conv((k + CV + 1) % R, (k + CV) % R, (k + CV - 1) % R, (k + CV) % R)
                elif fn == 0:
                    conv((k + CV + 1) % R, (k + CV) % R, (k + CV - 1) % R, (k + CV) % R, k % 2)
                elif fn == 2:
                    conv((k + CV + 1) % R, (k + CV) % R, (k + CV - 1) % R, (k + CV) % R, (k + 1) % 2)
                elif fn == 4:
                    m, jA, jB = o.get('m', 4), o.get('jA', 2), o.get('jB', 0)
                    def mk(kk_):
                        fA = (lambda: V['tb'][kk_ % 2][jA]) if (jA >= 0 and kk_ > 0) else None
                        fB = (lambda: V['tb'][(kk_ + 1) % 2][jB]) if jB >= 0 else None
                        return convg((kk_ + CV + 1) % R, (kk_ + CV) % R, (kk_ + CV - 1) % R, (kk_ + CV) % R, None, m, fA, fB)
                    if k == 0:
                        pend = mk(0)
                        next(pend)
                    for _ in pend:
                        pass
                    if k + 1 < R:
                        pend = mk(k + 1)
                        next(pend)
                elif fn == 3:
                    conv((k + CV + 1) % R, (k + CV) % R, (k + CV - 1) % R, (k + CV) % R, (k + 1) % 2 if k > 0 else None)
                mm1((k + 1) % R, (k + 1) % 2)
                if fn == 1 and k > 0:
                    kp = k - 1
                    conv((kp + CV + 1) % R, (kp + CV) % R, (kp + CV - 1) % R, (kp + CV) % R, k % 2)
                mm2(k % 2, k, os_ * R + k)
                if fn == 1 and k == R - 1:
                    conv((k + CV + 1) % R, (k + CV) % R, (k + CV - 1) % R, (k + CV) % R)
                if (k + 1) % OQ == 0:
                    out_copy(gi, oslot, k // OQ).start()
            return carry

        NGR = o.get('ng', NG)
        if PK:
            body(0, 0, True)
        lax.fori_loop(1 if PK else 0, NGR, body, 0)
        in_copy(0, NGR % NXB).wait()
        for gi in range(NGR - NOB, NGR):
            for q in range(NQ):
                out_copy(gi, gi % NOB, q).wait()

    return kernel


def build(o, name="cnx"):
    kern = make_kernel(o)
    R = o.get('R', 16)
    NQ = R // o.get('oq', 4)

    def f(x, dw, w1, b1, w2, b2, gamma):
        xt = jnp.transpose(x, (0, 1, 3, 2)).reshape(H, C, W)
        out = pl.pallas_call(
            kern,
            out_shape=jax.ShapeDtypeStruct((H, C, W), BF16),
            in_specs=[pl.BlockSpec(memory_space=pl.ANY)] + [pl.BlockSpec(memory_space=pltpu.VMEM)] * 6,
            out_specs=pl.BlockSpec(memory_space=pl.ANY),
            scratch_shapes=[
                pltpu.VMEM((NXB * R + 8, C, W), BF16), pltpu.VMEM((NOB * R, C, W), BF16),
                pltpu.VMEM((R, C, W), F32), pltpu.VMEM((R, C, W), F32), pltpu.VMEM((R, 8, 128), F32),
                pltpu.VMEM((E, W), U32), pltpu.VMEM((2 * E, W), F32),
                pltpu.VMEM((E // 2 + 24, W), U32), pltpu.VMEM((E // 2 + 24, W), U32)] + [pltpu.VMEM((64 + 24, W), U32)] * 6 + [pltpu.SMEM((2,), jnp.int32),
                pltpu.VMEM((9, C, 128), F32), pltpu.VMEM((32, 128), F32),
                pltpu.VMEM((E // 2, 128), U32), pltpu.VMEM((C // 2, E), U32),
                pltpu.VMEM((C, 128), F32),
                pltpu.SemaphoreType.DMA((2 * NXB + 1,)), pltpu.SemaphoreType.DMA((NOB * NQ,))],
            compiler_params=pltpu.CompilerParams(vmem_limit_bytes=100 * 1024 * 1024, flags=o.get('flags'),
                                                 disable_bounds_checks=o.get('dbc', True)),
            name=name,
        )(xt, dw, w1, b1, w2.T, b2, gamma)
        return jnp.transpose(out.reshape(1, H, C, W), (0, 1, 3, 2))
    return f


_impl = build({'R': 32, 'gp': 1, 'ko': 1, 'fo': 1, 'cvs': 2, 'cs': 0, 'po': 1, 'yo': 1, 'ge': 0, 'cw': 16, 'to': 1, 'cts': 2, 'cf': 0, 'wa': 0, 'lv': 0,'peel':8,'upro':1})


@jax.jit
def pallas_standalone__modern_conv_block_convnext__vision_kernel(x, dw, w1, b1, w2, b2, gamma):
    return _impl(x, dw, w1, b1, w2, b2, gamma)
```

```python
import numpy as np
import jax
import jax.numpy as jnp
from jax import lax
import jax.experimental.pallas as pl
import jax.experimental.pallas.tpu as pltpu

F32 = jnp.float32
BF16 = jnp.bfloat16
U32 = jnp.uint32

H = W = 512
C = 96
E = 384
NT = W // 128
NC = C // 8
R = 32
NG = H // R
CV = 3
CT = 6
OQ = 4
NQ = R // OQ
PK = 8
EPS = 1e-5
C1 = float(np.sqrt(2.0 / np.pi))
C2 = C1 * 0.044715
GA = float(C2 ** (1.0 / 3.0))
GK = C1 / GA
DN = (((1,), (0,)), ((), ()))


class _Copies:
    def __init__(self, *copies):
        self.copies = copies

    def start(self):
        for c in self.copies:
            c.start()

    def wait(self):
        for c in self.copies:
            c.wait()


def _kernel(x_hbm, dw_ref, w1_ref, b1_ref, w2t_ref, b2_ref, g_ref, o_hbm,
            xbuf, obuf, ring, cb, rb, gbuf, wdw, cst, w1t, w2s, bias2, isem, osem):

    def in_copy(g, slot):
        a0 = jnp.minimum(g * R + CT, H - R + CT)
        b0 = jnp.minimum((g + 1) * R, H - CT)
        return _Copies(
            pltpu.make_async_copy(x_hbm.at[pl.ds(a0, R - CT)], xbuf.at[pl.ds(slot * R, R - CT)], isem.at[2 * slot]),
            pltpu.make_async_copy(x_hbm.at[pl.ds(b0, CT)], xbuf.at[pl.ds(slot * R + R - CT, CT)], isem.at[2 * slot + 1]))

    def out_copy(g, slot, q):
        return pltpu.make_async_copy(obuf.at[pl.ds(slot * R + q * OQ, OQ)], o_hbm.at[pl.ds(g * R + q * OQ, OQ)],
                                     osem.at[slot * NQ + q])

    first = pltpu.make_async_copy(x_hbm.at[pl.ds(0, CT)], xbuf.at[pl.ds(2 * R, CT)], isem.at[4])
    p0 = pltpu.make_async_copy(x_hbm.at[pl.ds(CT, PK)], xbuf.at[pl.ds(0, PK)], isem.at[0])
    p1 = pltpu.make_async_copy(x_hbm.at[pl.ds(CT + PK, R - PK)], xbuf.at[pl.ds(PK, R - PK)], isem.at[1])
    first.start()
    p0.start()
    p1.start()

    dwp = dw_ref[...].astype(F32).reshape(9, C)
    dwp = jnp.concatenate([dwp, jnp.zeros((128 - 9, C), F32)], axis=0)
    dwp = jnp.concatenate([dwp, jnp.zeros((128, 128 - C), F32)], axis=1)
    dwt = dwp.T
    for k in range(9):
        wdw[k] = jnp.broadcast_to(dwt[:C, k:k + 1], (C, 128))
    w1 = w1_ref[...].astype(F32)
    w1c = w1 - jnp.mean(w1, axis=0, keepdims=True)
    b1 = b1_ref[...].astype(F32).reshape(1, E) * GA
    bh = b1.astype(BF16).astype(F32)
    ext = jnp.concatenate([bh, b1 - bh, jnp.zeros((128 - C - 2, E), F32)], axis=0)
    w1t[...] = pltpu.bitcast(jnp.concatenate([w1c, ext], axis=0).T.astype(BF16), U32)
    gam = g_ref[...].astype(F32).reshape(1, C)
    gb2 = gam * b2_ref[...].astype(F32).reshape(1, C)
    gg = jnp.concatenate([gam * (0.5 / GA), gb2, jnp.zeros((126, C), F32)], axis=0)
    gg = jnp.concatenate([gg, jnp.zeros((128, 128 - C), F32)], axis=1)
    ggt = gg.T
    gcol = jnp.broadcast_to(ggt[:C, 0:1], (C, E))
    w2s[...] = pltpu.bitcast((w2t_ref[...].astype(F32) * gcol).astype(BF16), U32)
    bias2[...] = jnp.broadcast_to(ggt[:C, 1:2], (C, 128))
    rowi = lax.broadcasted_iota(jnp.int32, (32, 128), 0)
    cst[...] = jnp.where(rowi < 2, 1.0, 0.0)

    sub = lax.broadcasted_iota(jnp.int32, (8, 128), 0)
    lane = lax.broadcasted_iota(jnp.int32, (8, 128), 1)
    m0 = lane == 0
    m127 = lane == 127

    def cvt(xidx, slot, valid):
        for c in range(C // 16):
            v = xbuf[xidx, pl.ds(c * 16, 16), :].astype(F32)
            if valid is not None:
                v = jnp.where(valid, v, 0.0)
            ring[slot, pl.ds(c * 16, 16), :] = v

    def conv(sl2, sl1, sl0, par):
        S = [None] * NT
        Q = [None] * NT
        for k in range(NC - 1, -1, -1):
            cs = pl.ds(k * 8, 8)
            w = [wdw[i, cs, :] for i in range(9)]
            r0, s1, l2 = [], [], []
            for t in range(NT):
                ls = pl.ds(t * 128, 128)
                a = ring[sl0, cs, ls]
                b = ring[sl1, cs, ls]
                c = ring[sl2, cs, ls]
                r0.append(pltpu.roll((a * w[0] + b * w[3]) + c * w[6], 1, 1))
                s1.append((a * w[1] + b * w[4]) + c * w[7])
                l2.append(pltpu.roll((a * w[2] + b * w[5]) + c * w[8], 127, 1))
            for t in range(NT - 1, -1, -1):
                lft = jnp.where(m0, r0[t - 1] if t > 0 else 0.0, r0[t])
                rgt = jnp.where(m127, l2[t + 1] if t < NT - 1 else 0.0, l2[t])
                v = (lft + rgt) + s1[t]
                cb[par, cs, pl.ds(t * 128, 128)] = v
                if S[t] is None:
                    S[t] = v
                    Q[t] = v * v
                else:
                    S[t] = S[t] + v
                    Q[t] = Q[t] + v * v

        def merge(a, b, d):
            msk = (sub % (2 * d)) < d
            return jnp.where(msk, a, b) + pltpu.roll(jnp.where(msk, b, a), 8 - d, 0)
        v = merge(merge(merge(S[0], S[1], 1), merge(S[2], S[3], 1), 2),
                  merge(merge(Q[0], Q[1], 1), merge(Q[2], Q[3], 1), 2), 4) * (1.0 / C)
        var = pltpu.roll(v, 4, 0) - v * v
        rb[par] = lax.rsqrt(jnp.maximum(var, 0.0) + EPS) * GA

    def mm1(par, gsl):
        r = jnp.concatenate([jnp.broadcast_to(rb[par, pl.ds(t, 1), :], (8, 128)) for t in range(NT)], axis=1)
        c32 = cst[...]
        xn = jnp.concatenate(
            [cb[par, pl.ds(c * 8, 8), :] * r for c in range(NC)] + [jnp.concatenate([c32] * NT, axis=1)], axis=0)
        h = lax.dot_general(pltpu.bitcast(w1t[...], BF16), xn, DN, preferred_element_type=F32)
        z = h * (h * h + GK)
        g = (jnp.tanh(z) + 1.0) * h
        gbuf[pl.ds(gsl * (E // 2), E // 2), :] = pltpu.bitcast(g.astype(BF16), U32)

    def mm2(gsl, rslot, oidx):
        def d(k0, kl, n0):
            g = pltpu.bitcast(gbuf[pl.ds(gsl * (E // 2) + k0 // 2, kl // 2), pl.ds(n0, 256)], BF16)
            return lax.dot_general(pltpu.bitcast(w2s[:, k0:k0 + kl], BF16), g, DN, preferred_element_type=F32)

        def half(n0, ka, kb):
            ya = d(*ka, n0)
            ts = []
            for c in range(NC):
                cs = pl.ds(c * 8, 8)
                b = jnp.concatenate([bias2[cs, :]] * 2, axis=1)
                ts.append((ya[c * 8:c * 8 + 8, :] + ring[rslot, cs, pl.ds(n0, 256)]) + b)
            yb = d(*kb, n0)
            for c in range(NC):
                obuf[oidx, pl.ds(c * 8, 8), pl.ds(n0, 256)] = (ts[c] + yb[c * 8:c * 8 + 8, :]).astype(BF16)
        half(0, (128, 256), (0, 128))
        half(256, (256, 128), (0, 256))

    ring[R - 1] = jnp.zeros((C, W), F32)
    first.wait()
    for r in range(CT):
        cvt(2 * R + r, r, None)
    for r in range(CV):
        conv(r + 1, r, (r + R - 1) % R, r)
    mm1(0, 0)

    def body(gi, carry, peeled=False):
        slot = gi % 2
        in_copy(jnp.minimum(gi + 1, NG - 1), (gi + 1) % 2).start()
        if peeled:
            p0.wait()
        else:
            @pl.when(gi >= 2)
            def _():
                for q in range(NQ):
                    out_copy(0, slot, q).wait()
            in_copy(0, slot).wait()

        for k in range(R):
            if peeled and k == PK:
                p1.wait()
            valid = (gi * R + k + CT < H) if k + CT == R else None
            cvt(slot * R + k, (k + CT) % R, valid)
            conv((k + CV + 1) % R, (k + CV) % R, (k + CV - 1) % R, (k + CV) % R)
            mm1((k + 1) % R, (k + 1) % 2)
            mm2(k % 2, k, slot * R + k)
            if (k + 1) % OQ == 0:
                out_copy(gi, slot, k // OQ).start()
        return carry

    body(0, 0, True)
    lax.fori_loop(1, NG, body, 0)
    in_copy(0, NG % 2).wait()
    for gi in range(NG - 2, NG):
        for q in range(NQ):
            out_copy(gi, gi % 2, q).wait()


@jax.jit
def pallas_standalone__modern_conv_block_convnext__vision_kernel(
    x: jax.Array,
    dw: jax.Array,
    w1: jax.Array,
    b1: jax.Array,
    w2: jax.Array,
    b2: jax.Array,
    gamma: jax.Array,
):
    xt = jnp.transpose(x, (0, 1, 3, 2)).reshape(H, C, W)
    vmem = pl.BlockSpec(memory_space=pltpu.VMEM)
    out = pl.pallas_call(
        _kernel,
        out_shape=jax.ShapeDtypeStruct((H, C, W), BF16),
        in_specs=[pl.BlockSpec(memory_space=pl.ANY)] + [vmem] * 6,
        out_specs=pl.BlockSpec(memory_space=pl.ANY),
        scratch_shapes=[
            pltpu.VMEM((2 * R + 8, C, W), BF16),
            pltpu.VMEM((2 * R, C, W), BF16),
            pltpu.VMEM((R, C, W), F32),
            pltpu.VMEM((R, C, W), F32),
            pltpu.VMEM((R, 8, 128), F32),
            pltpu.VMEM((E, W), U32),
            pltpu.VMEM((9, C, 128), F32),
            pltpu.VMEM((32, 128), F32),
            pltpu.VMEM((E // 2, 128), U32),
            pltpu.VMEM((C // 2, E), U32),
            pltpu.VMEM((C, 128), F32),
            pltpu.SemaphoreType.DMA((5,)),
            pltpu.SemaphoreType.DMA((2 * NQ,)),
        ],
        compiler_params=pltpu.CompilerParams(vmem_limit_bytes=100 * 1024 * 1024, disable_bounds_checks=True),
        name="convnext_block",
    )(xt, dw, w1, b1, w2.T, b2, gamma)
    return jnp.transpose(out.reshape(1, H, C, W), (0, 1, 3, 2))
```

```python
import numpy as np
import jax
import jax.numpy as jnp
from jax import lax
import jax.experimental.pallas as pl
import jax.experimental.pallas.tpu as pltpu

F32 = jnp.float32
BF16 = jnp.bfloat16
U32 = jnp.uint32

H = W = 512
C = 96
E = 384
NT = W // 128
NC = C // 8
R = 32
NG = H // R
CV = 3
CT = 5
OQ = 4
NQ = R // OQ
PK = 8
EPS = 1e-5
C1 = float(np.sqrt(2.0 / np.pi))
C2 = C1 * 0.044715
GA = float(C2 ** (1.0 / 3.0))
GK = C1 / GA
DN = (((1,), (0,)), ((), ()))


class _Copies:
    def __init__(self, *copies):
        self.copies = copies

    def start(self):
        for c in self.copies:
            c.start()

    def wait(self):
        for c in self.copies:
            c.wait()


def _kernel(x_hbm, dw_ref, w1_ref, b1_ref, w2t_ref, b2_ref, g_ref, o_hbm,
            xbuf, obuf, ring, cb, rb, gbuf, wdw, cst, w1t, w2s, bias2, isem, osem):

    def in_copy(g, slot):
        a0 = jnp.minimum(g * R + CT, H - R + CT)
        b0 = jnp.minimum((g + 1) * R, H - CT)
        return _Copies(
            pltpu.make_async_copy(x_hbm.at[pl.ds(a0, R - CT)], xbuf.at[pl.ds(slot * R, R - CT)], isem.at[2 * slot]),
            pltpu.make_async_copy(x_hbm.at[pl.ds(b0, CT)], xbuf.at[pl.ds(slot * R + R - CT, CT)], isem.at[2 * slot + 1]))

    def out_copy(g, slot, q):
        return pltpu.make_async_copy(obuf.at[pl.ds(slot * R + q * OQ, OQ)], o_hbm.at[pl.ds(g * R + q * OQ, OQ)],
                                     osem.at[slot * NQ + q])

    first = pltpu.make_async_copy(x_hbm.at[pl.ds(0, CT)], xbuf.at[pl.ds(2 * R, CT)], isem.at[4])
    p0 = pltpu.make_async_copy(x_hbm.at[pl.ds(CT, PK)], xbuf.at[pl.ds(0, PK)], isem.at[0])
    p1 = pltpu.make_async_copy(x_hbm.at[pl.ds(CT + PK, R - PK)], xbuf.at[pl.ds(PK, R - PK)], isem.at[1])
    first.start()
    p0.start()
    p1.start()

    dwp = dw_ref[...].astype(F32).reshape(9, C)
    dwp = jnp.concatenate([dwp, jnp.zeros((128 - 9, C), F32)], axis=0)
    dwp = jnp.concatenate([dwp, jnp.zeros((128, 128 - C), F32)], axis=1)
    dwt = dwp.T
    for k in range(9):
        wdw[k] = jnp.broadcast_to(dwt[:C, k:k + 1], (C, 128))
    w1 = w1_ref[...].astype(F32)
    w1c = w1 - jnp.mean(w1, axis=0, keepdims=True)
    b1 = b1_ref[...].astype(F32).reshape(1, E) * GA
    bh = b1.astype(BF16).astype(F32)
    ext = jnp.concatenate([bh, b1 - bh, jnp.zeros((128 - C - 2, E), F32)], axis=0)
    w1t[...] = pltpu.bitcast(jnp.concatenate([w1c, ext], axis=0).T.astype(BF16), U32)
    gam = g_ref[...].astype(F32).reshape(1, C)
    gb2 = gam * b2_ref[...].astype(F32).reshape(1, C)
    gg = jnp.concatenate([gam * (0.5 / GA), gb2, jnp.zeros((126, C), F32)], axis=0)
    gg = jnp.concatenate([gg, jnp.zeros((128, 128 - C), F32)], axis=1)
    ggt = gg.T
    gcol = jnp.broadcast_to(ggt[:C, 0:1], (C, E))
    w2s[...] = pltpu.bitcast((w2t_ref[...].astype(F32) * gcol).astype(BF16), U32)
    bias2[...] = jnp.broadcast_to(ggt[:C, 1:2], (C, 128))
    rowi = lax.broadcasted_iota(jnp.int32, (32, 128), 0)
    cst[...] = jnp.where(rowi < 2, 1.0, 0.0)

    sub = lax.broadcasted_iota(jnp.int32, (8, 128), 0)
    lane = lax.broadcasted_iota(jnp.int32, (8, 128), 1)
    m0 = lane == 0
    m127 = lane == 127

    def cvt(xidx, slot, valid):
        for c in range(NC):
            v = xbuf[xidx, pl.ds(c * 8, 8), :].astype(F32)
            if valid is not None:
                v = jnp.where(valid, v, 0.0)
            ring[slot, pl.ds(c * 8, 8), :] = v

    def conv(sl2, sl1, sl0, par):
        S = [None] * NT
        Q = [None] * NT
        piv = [None] * NT
        for k in range(NC):
            cs = pl.ds(k * 8, 8)
            w = [wdw[i, cs, :] for i in range(9)]
            r0, s1, l2 = [], [], []
            for t in range(NT):
                ls = pl.ds(t * 128, 128)
                a = ring[sl0, cs, ls]
                b = ring[sl1, cs, ls]
                c = ring[sl2, cs, ls]
                r0.append(pltpu.roll((a * w[0] + b * w[3]) + c * w[6], 1, 1))
                s1.append((a * w[1] + b * w[4]) + c * w[7])
                l2.append(pltpu.roll((a * w[2] + b * w[5]) + c * w[8], 127, 1))
            for t in range(NT - 1, -1, -1):
                lft = jnp.where(m0, r0[t - 1] if t > 0 else 0.0, r0[t])
                rgt = jnp.where(m127, l2[t + 1] if t < NT - 1 else 0.0, l2[t])
                v = (s1[t] + lft) + rgt
                if piv[t] is None:
                    p = v
                    for d in (4, 2, 1):
                        p = p + pltpu.roll(p, d, 0)
                    piv[t] = p * 0.125
                v = v - piv[t]
                cb[par, cs, pl.ds(t * 128, 128)] = v
                if S[t] is None:
                    S[t] = v
                    Q[t] = v * v
                else:
                    S[t] = v + S[t]
                    Q[t] = v * v + Q[t]

        def merge(a, b, d):
            msk = (sub % (2 * d)) < d
            return jnp.where(msk, a, b) + pltpu.roll(jnp.where(msk, b, a), 8 - d, 0)
        v = merge(merge(merge(S[0], S[1], 1), merge(S[2], S[3], 1), 2),
                  merge(merge(Q[0], Q[1], 1), merge(Q[2], Q[3], 1), 2), 4) * (1.0 / C)
        var = pltpu.roll(v, 4, 0) - v * v
        rb[par] = lax.rsqrt(jnp.maximum(var, 0.0) + EPS) * GA

    def mm1(par, gsl):
        r = jnp.concatenate([jnp.broadcast_to(rb[par, pl.ds(t, 1), :], (8, 128)) for t in range(NT)], axis=1)
        c32 = cst[...]
        xn = jnp.concatenate(
            [cb[par, pl.ds(c * 8, 8), :] * r for c in range(NC)] + [jnp.concatenate([c32] * NT, axis=1)], axis=0)
        h = lax.dot_general(pltpu.bitcast(w1t[...], BF16), xn, DN, preferred_element_type=F32)
        z = (h * h + GK) * h
        g = h * (1.0 + jnp.tanh(z))
        gbuf[pl.ds(gsl * (E // 2), E // 2), :] = pltpu.bitcast(g.astype(BF16), U32)

    def mm2(gsl, rslot, oidx):
        def d(k0, kl, n0):
            g = pltpu.bitcast(gbuf[pl.ds(gsl * (E // 2) + k0 // 2, kl // 2), pl.ds(n0, 256)], BF16)
            return lax.dot_general(pltpu.bitcast(w2s[:, k0:k0 + kl], BF16), g, DN, preferred_element_type=F32)

        def half(n0, ka, kb):
            ya = d(*ka, n0)
            ts = []
            for c in range(NC):
                cs = pl.ds(c * 8, 8)
                b = jnp.concatenate([bias2[cs, :]] * 2, axis=1)
                ts.append(ya[c * 8:c * 8 + 8, :] + (ring[rslot, cs, pl.ds(n0, 256)] + b))
            yb = d(*kb, n0)
            for c in range(NC):
                obuf[oidx, pl.ds(c * 8, 8), pl.ds(n0, 256)] = (ts[c] + yb[c * 8:c * 8 + 8, :]).astype(BF16)
        half(0, (128, 256), (0, 128))
        half(256, (256, 128), (0, 256))

    ring[R - 1] = jnp.zeros((C, W), F32)
    first.wait()
    for r in range(CT):
        cvt(2 * R + r, r, None)
    for r in range(CV):
        conv(r + 1, r, (r + R - 1) % R, r)
    mm1(0, 0)

    def body(gi, carry, peeled=False):
        slot = gi % 2
        in_copy(jnp.minimum(gi + 1, NG - 1), (gi + 1) % 2).start()
        if peeled:
            p0.wait()
        else:
            @pl.when(gi >= 2)
            def _():
                for q in range(NQ):
                    out_copy(0, slot, q).wait()
            in_copy(0, slot).wait()

        for k in range(R):
            if peeled and k == PK:
                p1.wait()
            valid = (gi * R + k + CT < H) if k + CT == R else None
            cvt(slot * R + k, (k + CT) % R, valid)
            conv((k + CV + 1) % R, (k + CV) % R, (k + CV - 1) % R, (k + CV) % R)
            mm1((k + 1) % R, (k + 1) % 2)
            mm2(k % 2, k, slot * R + k)
            if (k + 1) % OQ == 0:
                out_copy(gi, slot, k // OQ).start()
        return carry

    body(0, 0, True)
    lax.fori_loop(1, NG, body, 0)
    in_copy(0, NG % 2).wait()
    for gi in range(NG - 2, NG):
        for q in range(NQ):
            out_copy(gi, gi % 2, q).wait()


@jax.jit
def pallas_standalone__modern_conv_block_convnext__vision_kernel(
    x: jax.Array,
    dw: jax.Array,
    w1: jax.Array,
    b1: jax.Array,
    w2: jax.Array,
    b2: jax.Array,
    gamma: jax.Array,
):
    xt = jnp.transpose(x, (0, 1, 3, 2)).reshape(H, C, W)
    vmem = pl.BlockSpec(memory_space=pltpu.VMEM)
    out = pl.pallas_call(
        _kernel,
        out_shape=jax.ShapeDtypeStruct((H, C, W), BF16),
        in_specs=[pl.BlockSpec(memory_space=pl.ANY)] + [vmem] * 6,
        out_specs=pl.BlockSpec(memory_space=pl.ANY),
        scratch_shapes=[
            pltpu.VMEM((2 * R + 8, C, W), BF16),
            pltpu.VMEM((2 * R, C, W), BF16),
            pltpu.VMEM((R, C, W), F32),
            pltpu.VMEM((R, C, W), F32),
            pltpu.VMEM((R, 8, 128), F32),
            pltpu.VMEM((E, W), U32),
            pltpu.VMEM((9, C, 128), F32),
            pltpu.VMEM((32, 128), F32),
            pltpu.VMEM((E // 2, 128), U32),
            pltpu.VMEM((C // 2, E), U32),
            pltpu.VMEM((C, 128), F32),
            pltpu.SemaphoreType.DMA((5,)),
            pltpu.SemaphoreType.DMA((2 * NQ,)),
        ],
        compiler_params=pltpu.CompilerParams(vmem_limit_bytes=100 * 1024 * 1024, disable_bounds_checks=True),
        name="convnext_block",
    )(xt, dw, w1, b1, w2.T, b2, gamma)
    return jnp.transpose(out.reshape(1, H, C, W), (0, 1, 3, 2))
```
